```python
import os as _os
_os.environ.setdefault("JAX_PLATFORMS", "cpu")
import jax
import jax.numpy as jnp

def _softmax(x, axis=-1):
    return jax.nn.softmax(x, axis=axis)
def _gelu(x):
    return jax.nn.gelu(x, approximate=True)
def _silu(x):
    return jax.nn.silu(x)
def _sigmoid(x):
    return jax.nn.sigmoid(x)
def _layernorm(x, axis=-1, eps=1e-5):
    m = jnp.mean(x, axis=axis, keepdims=True)
    v = jnp.var(x, axis=axis, keepdims=True)
    return (x - m) / jnp.sqrt(v + eps)
def _scatter_add(tgt, idx, src, axis=0):
    return tgt.at[idx].add(src)
def _segment_sum(src, seg, n):
    return jax.ops.segment_sum(src, seg, n)
class _Rng:
    def __init__(self, key):
        self._k = key
    def _next(self):
        self._k, sub = jax.random.split(self._k)
        return sub
    def normal(self, shape):
        return jax.random.normal(self._next(), shape, dtype=jnp.bfloat16)
    def randint(self, lo, hi, shape):
        return jax.random.randint(self._next(), shape, lo, hi, dtype=jnp.int32)
    def uniform(self, shape, lo=0.0, hi=1.0):
        return jax.random.uniform(self._next(), shape, jnp.bfloat16, lo, hi)
    def permutation(self, n):
        return jax.random.permutation(self._next(), n)


kernel_name = 'parallel_sum__sliding_local_dilated__dense_activation_mish__prompt'

def setup_inputs():
    _rng = _Rng(jax.random.key(int.from_bytes(__import__("os").urandom(4), "little")))
    _w = (lambda a: (lambda t: t.astype(jnp.bfloat16) if jnp.issubdtype(t.dtype, jnp.floating) else t)(jnp.asarray(a)))
    def _A_setup():
        B, S, D = 1, 2048, 576
        return {
            "x": _w((lambda *s: _rng.normal(s) * 0.05)(B, S, D)),
            "wqkv": _w((lambda *s: _rng.normal(s) * 0.05)(D, 3 * D)),
            "wo": _w((lambda *s: _rng.normal(s) * 0.05)(D, D)),
        }
    _A_in = _A_setup()

    def _B_setup():
        B, S, D, F = 1, 2048, 576, 4608
        return {
            "x": _w((lambda *s: _rng.normal(s) * 0.05)(B, S, D)),
            "w1": _w((lambda *s: _rng.normal(s) * 1.6)(D, F) * (D ** -0.5)),
            "b1": _w((lambda *s: _rng.normal(s) * 0.2)(F)),
            "w2": _w((lambda *s: _rng.normal(s) * 0.2)(F, D) * (F ** -0.5)),
        }
    _B_in = _B_setup()

    return {
        "A_x": _A_in["x"],
        "A_wqkv": _A_in["wqkv"],
        "A_wo": _A_in["wo"],
        "B_x": _B_in["x"],
        "B_w1": _B_in["w1"],
        "B_b1": _B_in["b1"],
        "B_w2": _B_in["w2"],
    }

def reference(A_x, A_wqkv, A_wo, B_x, B_w1, B_b1, B_w2):
    def _A_ref(x, wqkv, wo):
        B, S, D = x.shape
        H = 32; Dh = D // H
        W, dil = 8, 2
        qkv = (lambda x, *d: x.transpose(*d))((x @ wqkv).reshape(B, S, 3, H, Dh), 2, 0, 3, 1, 4)
        q, k, v = qkv[0], qkv[1], qkv[2]
        scale = Dh ** -0.5
        pos = jnp.arange(S)
        off = jnp.arange(W) * dil
        idx = pos[:, None] - off[None, :]
        mask = idx >= 0
        idx_c = jnp.where(mask, idx, 0).reshape(-1)
        kg = k[:, :, idx_c, :].reshape(B, H, S, W, Dh)
        vg = v[:, :, idx_c, :].reshape(B, H, S, W, Dh)
        logits = jnp.einsum("bhsd,bhswd->bhsw", q, kg) * scale
        logits = jnp.where(mask[None, None, :, :], logits, -1e9)
        attn = _softmax(logits, axis=-1)
        o = jnp.einsum("bhsw,bhswd->bhsd", attn, vg)
        return (lambda x, *d: x.transpose(*d))(o, 0, 2, 1, 3).reshape(B, S, D) @ wo

    def _B_ref(x, w1, b1, w2):
        h = jnp.einsum("bsd,df->bsf", x, w1) + b1
        sp = jnp.log1p(jnp.exp(-jnp.abs(h))) + jnp.where(h > 0, h, jnp.zeros_like(h))
        act = h * jnp.tanh(sp)
        return jnp.einsum("bsf,fd->bsd", act, w2)

    x = A_x
    xn = _layernorm(x, axis=-1)
    return x + _A_ref(xn, A_wqkv, A_wo) + _B_ref(xn, B_w1, B_b1, B_w2)
```

```python
import functools
import jax, jax.numpy as jnp
import jax.experimental.pallas as pl
import jax.experimental.pallas.tpu as pltpu

S, D, F = 2048, 576, 4608
H, DH, W, DIL = 32, 18, 8, 2
T = 512
NTILE = S // T
TF = 512
NC = F // TF
HALO = 16
NQKV = 1792
LOG2E = 1.4426950408889634
SCALE = DH ** -0.5
f32, bf16, i32 = jnp.float32, jnp.bfloat16, jnp.int32
NT = (((1,), (1,)), ((), ()))

def mish(h):
    u = jnp.exp(jnp.minimum(h, 20.0))
    n = u * (u + 2.0)
    return h * (n * pl.reciprocal(n + 2.0, approx=True))

def wp_row(part, d):
    if d < 16:
        return part * 512 + d * 32
    base = {0: 1536, 2: 1600, 1: 1664}[part]
    return base + (d - 16) * 32

def store_tiles(s, val):
    n = val.shape[1]
    for i in range(s.shape[0]):
        w = min(128, n - 128 * i)
        s[i, :, :w] = val[:, 128 * i:128 * i + w]

def load_strided(s, start, n, stride, width):
    parts = []
    for i in range(s.shape[0]):
        w = min(128, width - 128 * i)
        parts.append(s[i, pl.ds(start, n, stride=stride), :][:, :w])
    return jnp.concatenate(parts, axis=1)

def prep_weights(wqkv_v, wo_v, wt_s, wp_s, wof_s, wop_s):
    store_tiles(wt_s, wqkv_v[...].T.astype(f32))
    for part in range(3):
        for d in range(DH):
            rows = load_strided(wt_s, part * D + d, H, DH, D)
            wp_s[pl.ds(wp_row(part, d), H), :] = rows.astype(bf16)
    wp_s[pl.ds(1728, 64), :] = jnp.zeros((64, D), bf16)
    store_tiles(wof_s, wo_v[...].astype(f32))
    pieces = [load_strided(wof_s, d, H, DH, D).astype(bf16) for d in range(16)]
    pieces.append(jnp.zeros((64, D), bf16))
    pieces += [load_strided(wof_s, d, H, DH, D).astype(bf16) for d in (16, 17)]
    wop = jnp.concatenate(pieces, axis=0)
    wop_s[...] = wop.T

def kern(xt_hbm, wqkv_hbm, wo_hbm, w1_hbm, b1_hbm, w2t_hbm, out_hbm,
         x_v, wqkv_v, wo_v, w1_v, b1_v, w2_v, xn_s, acc_s, wt_s, wp_s, wof_s, wop_s,
         qkv_s, o_s, out_v, z_s, sem_x, sem_w1, sem_w2, sem_m, sem_o, *, mode):
    def cx(t):
        return pltpu.make_async_copy(xt_hbm.at[:, pl.ds(t * T, T)], x_v.at[:, pl.ds(t * T, T)], sem_x.at[t])
    def c1(c):
        return pltpu.make_async_copy(w1_hbm.at[:, pl.ds(c * TF, TF)], w1_v.at[:, pl.ds(c * TF, TF)], sem_w1.at[c])
    def c2(c):
        return pltpu.make_async_copy(w2t_hbm.at[:, pl.ds(c * TF, TF)], w2_v.at[:, pl.ds(c * TF, TF)], sem_w2.at[c])
    cb = pltpu.make_async_copy(b1_hbm, b1_v, sem_m.at[0])
    cq = pltpu.make_async_copy(wqkv_hbm, wqkv_v, sem_m.at[1])
    co = pltpu.make_async_copy(wo_hbm, wo_v, sem_m.at[2])
    def cout(t):
        return pltpu.make_async_copy(out_v.at[:, pl.ds(t * T, T)], out_hbm.at[:, pl.ds(t * T, T)], sem_o.at[t])

    cx(0).start(); cb.start(); c1(0).start(); c2(0).start()
    for t in range(1, NTILE):
        cx(t).start()
    cq.start(); co.start()
    c1(1).start(); c2(1).start()
    c1r = pltpu.make_async_copy(w1_hbm.at[:, pl.ds(2 * TF, F - 2 * TF)], w1_v.at[:, pl.ds(2 * TF, F - 2 * TF)], sem_w1.at[2])
    c2r = pltpu.make_async_copy(w2t_hbm.at[:, pl.ds(2 * TF, F - 2 * TF)], w2_v.at[:, pl.ds(2 * TF, F - 2 * TF)], sem_w2.at[2])
    c1r.start(); c2r.start()

    z_s[0] = 0
    for i in range(4, 14):
        qkv_s[i, pl.ds(T, HALO), :] = jnp.zeros((HALO, 128), f32)

    def tok_slice(t):
        return pl.ds(pl.multiple_of(t * T, T), T)

    def ln(t):
        xt = x_v[:, tok_slice(t)].astype(f32)
        m = jnp.mean(xt, axis=0, keepdims=True)
        xc = xt - m
        v = jnp.mean(xc * xc, axis=0, keepdims=True)
        xn_s[tok_slice(t), :] = (xc * jax.lax.rsqrt(v + 1e-5)).astype(bf16).T

    def ffn1(xnb, c):
        h = jnp.dot(xnb, w1_v[:, c * TF:(c + 1) * TF], preferred_element_type=f32)
        nb = TF // 128
        b = jnp.concatenate([b1_v[pl.ds(c * nb + i, 1), :] for i in range(nb)], axis=1)
        return mish(h + b.astype(f32)).astype(bf16)

    def ffn2(a, c):
        return jax.lax.dot_general(w2_v[:, c * TF:(c + 1) * TF], a, NT, preferred_element_type=f32)

    cx(0).wait()
    ln(0)
    cb.wait(); c1(0).wait()

    def p1_body(t, carry):
        a = ffn1(xn_s[tok_slice(t), :], 0)
        @pl.when(t == 0)
        def _():
            c2(0).wait()
        pltpu.make_async_copy(xt_hbm.at[:, tok_slice(t + 1)], x_v.at[:, tok_slice(t + 1)], sem_x.at[t + 1]).wait()
        acc_s[:, tok_slice(t)] = x_v[:, tok_slice(t)].astype(f32) + ffn2(a, 0)
        ln(t + 1)
        return carry
    jax.lax.fori_loop(0, NTILE - 1, p1_body, 0)

    tl = NTILE - 1
    cq.wait(); co.wait()
    a = ffn1(xn_s[tok_slice(tl), :], 0)
    prep_weights(wqkv_v, wo_v, wt_s, wp_s, wof_s, wop_s)
    acc_s[:, tok_slice(tl)] = x_v[:, tok_slice(tl)].astype(f32) + ffn2(a, 0)

    cexp = SCALE * LOG2E
    sub8 = jax.lax.broadcasted_iota(i32, (8, 128), 0)

    def p2_body(t, carry):
        @pl.when(t == 0)
        def _():
            c1(1).wait(); c2(1).wait()
        zvec = jnp.full((8, 128), z_s[0], i32)
        xnb = xn_s[tok_slice(t), :]
        acc = acc_s[:, tok_slice(t)] + ffn2(ffn1(xnb, 1), 1)
        for i in list(range(4, 14)):
            qkv_s[i, pl.ds(0, HALO), :] = qkv_s[i, pl.ds(T, HALO), :]
        qkv = jax.lax.dot_general(xnb, wp_s[...], NT, preferred_element_type=f32)
        for i in range(14):
            qkv_s[i, pl.ds(HALO, T), :] = qkv[:, 128 * i:128 * (i + 1)]
        @pl.when(t == 0)
        def _():
            c1r.wait(); c2r.wait()

        def ld(i, R):
            return qkv_s[i, pl.ds(R, 8), :]
        def gate(x, tok):
            return pltpu.bitcast(pltpu.bitcast(x, i32) | tok, f32)
        def token(x):
            return pltpu.bitcast(x, i32) & zvec

        def attn_row(j, tok):
            R = HALO + 8 * j
            q = [ld(i, R) for i in (0, 1, 2, 3, 12)]
            if tok is not None:
                q = [gate(x, tok) for x in q]
            s = []
            for w in range(W):
                Rw = R - DIL * w
                k = [ld(i, Rw) for i in (4, 5, 6, 7, 13)]
                sw = (q[0] * k[0] + q[1] * k[1]) + (q[2] * k[2] + q[3] * k[3]) + q[4] * k[4]
                sw = sw + pltpu.roll(sw, 64, 1)
                sw = sw + pltpu.roll(sw, 32, 1)
                if 8 * j < DIL * w:
                    valid = (sub8 + (t * T + 8 * j - DIL * w)) >= 0
                    sw = jnp.where(valid, sw, -1e9 / SCALE)
                s.append(sw)
            mx = functools.reduce(jnp.maximum, s)
            e = [jnp.exp2((sw - mx) * cexp) for sw in s]
            l = functools.reduce(lambda a, b: a + b, e)
            r = pl.reciprocal(l, approx=True)
            o = None
            for oi, i in enumerate((8, 9, 10, 11, 12)):
                ee = e
                if mode >= 1 and o is not None:
                    tk = token(o)
                    ee = [gate(x, tk) for x in e]
                pacc = None
                for w in range(W):
                    p = ee[w] * ld(i, R - DIL * w)
                    pacc = p if pacc is None else pacc + p
                o = pacc * r
                o_s[pl.ds(8 * j, 8), pl.ds(128 * oi, 128)] = o
            return token(o)

        tok = None
        for j in range(T // 8):
            tok = attn_row(j, tok)

        for c in range(2, NC):
            acc = acc + ffn2(ffn1(xnb, c), c)
        acc = acc + jax.lax.dot_general(wop_s[...], o_s[...].astype(bf16), NT, preferred_element_type=f32)
        out_v[:, tok_slice(t)] = acc.astype(bf16)
        pltpu.make_async_copy(out_v.at[:, tok_slice(t)], out_hbm.at[:, tok_slice(t)], sem_o.at[t]).start()
        return carry
    jax.lax.fori_loop(0, NTILE, p2_body, 0)
    for t in range(NTILE):
        cout(t).wait()

@jax.jit
def pallas_parallel_sum__sliding_local_dilated__dense_activation_mish__prompt_kernel(
    A_x: jax.Array,
    A_wqkv: jax.Array,
    A_wo: jax.Array,
    B_x: jax.Array,
    B_w1: jax.Array,
    B_b1: jax.Array,
    B_w2: jax.Array,
):
    del B_x
    xt = A_x.reshape(S, D).T
    anyspec = pl.BlockSpec(memory_space=pl.ANY)
    out = pl.pallas_call(
        functools.partial(kern, mode=1),
        in_specs=[anyspec] * 6,
        out_specs=anyspec,
        out_shape=jax.ShapeDtypeStruct((D, S), bf16),
        scratch_shapes=[
            pltpu.VMEM((D, S), bf16), pltpu.VMEM((D, 3 * D), bf16), pltpu.VMEM((D, D), bf16),
            pltpu.VMEM((D, F), bf16), pltpu.VMEM((F // 128, 128), bf16), pltpu.VMEM((D, F), bf16),
            pltpu.VMEM((S, D), bf16), pltpu.VMEM((D, S), f32),
            pltpu.VMEM((5, 3 * D, 128), f32), pltpu.VMEM((NQKV, D), bf16),
            pltpu.VMEM((5, D, 128), f32), pltpu.VMEM((D, 640), bf16),
            pltpu.VMEM((14, HALO + T, 128), f32), pltpu.VMEM((T, 640), f32),
            pltpu.VMEM((D, S), bf16), pltpu.SMEM((1,), i32),
            pltpu.SemaphoreType.DMA((NTILE,)), pltpu.SemaphoreType.DMA((NC,)), pltpu.SemaphoreType.DMA((NC,)),
            pltpu.SemaphoreType.DMA((3,)), pltpu.SemaphoreType.DMA((NTILE,)),
        ],
        compiler_params=pltpu.CompilerParams(vmem_limit_bytes=100 * 1024 * 1024),
    )(xt, A_wqkv, A_wo, B_w1, B_b1.reshape(F // 128, 128), B_w2.T)
    return out.T.reshape(1, S, D)
```

```python
import functools

import jax
import jax.numpy as jnp
import jax.experimental.pallas as pl
import jax.experimental.pallas.tpu as pltpu

S, D, F = 2048, 576, 4608
H, DH, W, DIL = 32, 18, 8, 2
T = 512
NTILE = S // T
NB = T // 128
HALO = 16
F0 = 768
FH = 256
CHUNKS = (768,) * 5
NPRE = 3
OSPLIT = (384, D)
NOD = NB - 1 + len(OSPLIT)
EPS = 1e-5
LOG2E = 1.4426950408889634
CEXP = DH ** -0.5 * LOG2E
NEG = -1e9 * LOG2E
f32, bf16, i32 = jnp.float32, jnp.bfloat16, jnp.int32
NT = (((1,), (1,)), ((), ()))


def _mish(h):
    u = jnp.exp(jnp.minimum(h, 20.0))
    n = u * (u + 2.0)
    return h * (n * pl.reciprocal(n + 2.0, approx=True))


def _gate(x, z, rows, dtype):
    if z is None:
        return x
    head = pltpu.bitcast(pltpu.bitcast(x[:rows, :128], i32) | z, dtype)
    if x.shape[1] > 128:
        head = jnp.concatenate([head, x[:rows, 128:]], axis=1)
    return jnp.concatenate([head, x[rows:]], axis=0) if x.shape[0] > rows else head


def _gate_f(x, z):
    return _gate(x, z, 8, f32)


def _gate_b(x, z):
    return _gate(x, z, 16, bf16)


def _wp_row(part, d):
    if d < 16:
        return part * 512 + d * 32
    return {0: 1536, 2: 1600, 1: 1664}[part] + (d - 16) * 32


def _gather_rows(s, start, width):
    parts = []
    for i in range(s.shape[0]):
        parts.append(s[i, pl.ds(start, H, stride=DH), :][:, :min(128, width - 128 * i)])
    return jnp.concatenate(parts, axis=1)


def _store_tiles(s, r0, val):
    for i in range(s.shape[0]):
        w = min(128, val.shape[1] - 128 * i)
        s[i, pl.ds(r0, val.shape[0]), :w] = val[:, 128 * i:128 * i + w]


def _prep_qkv(part, wqkv_v, wt_s, wp_s, zvec, z):
    lo = (part * D) // 128 * 128
    hi = min(-(-((part + 1) * D) // 128) * 128, 3 * D)
    for c0 in range(lo, hi, 128):
        cw = min(128, hi - c0)
        blk = wqkv_v[:, c0:c0 + cw]
        if cw == 128:
            blk = _gate_b(blk, z)
        wt = blk.T.astype(f32)
        _store_tiles(wt_s, c0 - lo, wt)
        z = pltpu.bitcast(wt[cw - 8:, 384:512], i32) & zvec
    for d in range(DH):
        rows = _gather_rows(wt_s, part * D - lo + d, D)
        if d % 3 == 0:
            rows = _gate_f(rows, z)
        rows = rows.astype(bf16)
        wp_s[pl.ds(_wp_row(part, d), H), :] = rows
        z = pltpu.bitcast(rows[:16, :128], i32) & zvec
    return z


def _prep_wo(wo_v, wof_s, wop_s, zvec):
    _store_tiles(wof_s, 0, wo_v[...].astype(f32))
    pieces = [_gather_rows(wof_s, d, D).astype(bf16) for d in range(16)]
    pieces.append(jnp.zeros((64, D), bf16))
    pieces += [_gather_rows(wof_s, d, D).astype(bf16) for d in (16, 17)]
    wopt = jnp.concatenate(pieces, axis=0).T
    wop_s[...] = wopt
    return (pltpu.bitcast(wopt[D - 16:, 512:], i32) | pltpu.bitcast(wopt[D - 16:, :128], i32)) & zvec


def _kernel(xt_hbm, wqkv_hbm, wo_hbm, w1_hbm, b1_hbm, w2t_hbm, out_hbm,
            x_v, wqkv_v, wo_v, w1_v, b1_v, w2_v, xn_s, acc_s, a_s, wt_s, wp_s, wof_s, wop_s,
            qkv_s, o_s, out_v, z_s, sem_in, sem_out):
    def cols(start, size):
        if isinstance(start, int):
            return pl.ds(start, size)
        return pl.ds(pl.multiple_of(start, 128), size)

    def tile(t):
        return cols(t * T, T)

    def cx(t):
        return pltpu.make_async_copy(xt_hbm.at[:, tile(t)], x_v.at[:, tile(t)], sem_in.at[8 + t])

    def cw(src, dst, lo, hi, k):
        return pltpu.make_async_copy(src.at[:, pl.ds(lo, hi - lo)], dst.at[:, pl.ds(lo, hi - lo)], sem_in.at[k])

    def out_copies(t, n):
        cs = cols(t * T + 128 * n, 128)
        if n < NB - 1:
            return [(0, D, pltpu.make_async_copy(out_v.at[:, cs], out_hbm.at[:, cs], sem_out.at[t * NOD + n]))]
        res, r0 = [], 0
        for k, r1 in enumerate(OSPLIT):
            res.append((r0, r1, pltpu.make_async_copy(out_v.at[r0:r1, cs], out_hbm.at[r0:r1, cs],
                                                      sem_out.at[t * NOD + n + k])))
            r0 = r1
        return res

    cb = pltpu.make_async_copy(b1_hbm, b1_v, sem_in.at[0])
    c1a = cw(w1_hbm, w1_v, 0, FH, 1)
    c1b = cw(w1_hbm, w1_v, FH, F0, 2)
    c2a = cw(w2t_hbm, w2_v, 0, F0, 3)
    cq = pltpu.make_async_copy(wqkv_hbm, wqkv_v, sem_in.at[4])
    co = pltpu.make_async_copy(wo_hbm, wo_v, sem_in.at[5])
    c1r = cw(w1_hbm, w1_v, F0, F, 6)
    c2r = cw(w2t_hbm, w2_v, F0, F, 7)
    for c in [cx(0), c1a, cb, c1b, c2a] + [cx(t) for t in range(1, NTILE)] + [cq, co, c1r, c2r]:
        c.start()

    z_s[0] = 0
    for i in range(4, 13):
        qkv_s[i, pl.ds(T, HALO), :] = jnp.zeros((HALO, 128), f32)
    qkv_s[13] = jnp.zeros((HALO + T, 128), f32)

    def zeros_vec():
        return jnp.full((8, 128), z_s[0], i32)

    def layernorm(start, ntok, blk):
        z = None
        for b in range(ntok // blk):
            sl = cols(start + blk * b, blk)
            xt = _gate_f(x_v[:, sl].astype(f32), z)
            xc = xt - jnp.mean(xt, axis=0, keepdims=True)
            v = jnp.mean(xc * xc, axis=0, keepdims=True)
            xn = (xc * jax.lax.rsqrt(v + EPS)).astype(bf16).T
            xn_s[sl, :] = xn
            z = (pltpu.bitcast(xn[blk - 16:, 384:512], i32) | pltpu.bitcast(xn[blk - 16:, :128], i32)) & zeros_vec()

    def bias(lo, hi):
        return jnp.concatenate([b1_v[pl.ds(i, 1), :] for i in range(lo // 128, hi // 128)], axis=1).astype(f32)

    def ffn1(xnb, lo, hi):
        return _mish(jnp.dot(xnb, w1_v[:, lo:hi], preferred_element_type=f32) + bias(lo, hi)).astype(bf16)

    def ffn1k(xnb, lo, hi, msplit):
        xa, xr = xnb[:, :512], xnb[:, 512:]
        mb = xnb.shape[0] // msplit
        rem = jnp.concatenate([jnp.dot(xr[i * mb:(i + 1) * mb], w1_v[512:, lo:hi], preferred_element_type=f32)
                               for i in range(msplit)], axis=0)
        outs = []
        for c0 in range(lo, hi, 128):
            h = jnp.dot(xa, w1_v[:512, c0:c0 + 128], preferred_element_type=f32)
            outs.append(_mish(h + (rem[:, c0 - lo:c0 - lo + 128] + bias(c0, c0 + 128))).astype(bf16))
        return jnp.concatenate(outs, axis=1)

    def ffn2(a, lo, hi):
        return jax.lax.dot_general(w2_v[:, lo:hi], a, NT, preferred_element_type=f32)

    def ffn2_first(t):
        w2c = w2_v[:, :F0]
        for n in range(NB):
            cs = cols(t * T + 128 * n, 128)
            acc_s[:, cs] = x_v[:, cs].astype(f32) + jax.lax.dot_general(
                w2c, a_s[128 * n:128 * (n + 1), :], NT, preferred_element_type=f32)

    HT = T // 2
    cx(0).wait()
    layernorm(0, HT, HT)
    c1a.wait()
    cb.wait()
    layernorm(HT, HT, HT)
    a_s[:HT, :FH] = ffn1k(xn_s[pl.ds(0, HT), :], 0, FH, 2)
    a_s[HT:, :FH] = ffn1k(xn_s[pl.ds(HT, HT), :], 0, FH, 2)
    c1b.wait()
    a_s[:, FH:] = ffn1k(xn_s[tile(0), :], FH, F0, 1)

    def p1_body(t, carry):
        @pl.when(t == 0)
        def _():
            c2a.wait()
        cx(t + 1).wait()
        layernorm((t + 1) * T, T, 128)
        ffn2_first(t)
        a_s[...] = ffn1k(xn_s[tile(t + 1), :], 0, F0, 2)
        return carry

    jax.lax.fori_loop(0, NTILE - 1, p1_body, 0)

    cq.wait()
    co.wait()
    zv = zeros_vec()
    z = _prep_wo(wo_v, wof_s, wop_s, zv)
    for part in range(3):
        z = _prep_qkv(part, wqkv_v, wt_s.at[part], wp_s, zv, z)
    ffn2_first(NTILE - 1)
    c1r.wait()
    c2r.wait()

    sub8 = jax.lax.broadcasted_iota(i32, (8, 128), 0)
    cexp_bits = pltpu.bitcast(jnp.full((8, 128), CEXP, f32), i32)

    def p2_body(t, carry):
        zvec = zeros_vec()
        xnb = xn_s[tile(t), :]
        bounds = [F0]
        for c in CHUNKS:
            bounds.append(bounds[-1] + c)
        acts = [ffn1(xnb, bounds[c], bounds[c + 1]) for c in range(NPRE)]

        for i in range(4, 14):
            qkv_s[i, pl.ds(0, HALO), :] = qkv_s[i, pl.ds(T, HALO), :]
        rem = jax.lax.dot_general(wp_s[pl.ds(1536, 192), :], xnb, NT, preferred_element_type=f32).T
        qkv_s[12, pl.ds(HALO, T), :] = rem[:, :128]
        qkv_s[13, pl.ds(HALO, T), :64] = rem[:, 128:]
        qkv = jax.lax.dot_general(xnb, wp_s[pl.ds(0, 1536), :], NT, preferred_element_type=f32)
        for i in range(12):
            qkv_s[i, pl.ds(HALO, T), :] = qkv[:, 128 * i:128 * (i + 1)]

        def ld(i, r):
            return qkv_s[i, pl.ds(r, 8), :]

        def token(x):
            return pltpu.bitcast(x, i32) & zvec

        def attn_rows(j, z):
            r = HALO + 8 * j
            scale = pltpu.bitcast(cexp_bits if z is None else cexp_bits | z, f32)
            q = [ld(i, r) * scale for i in (0, 1, 2, 3, 12)]
            s = []
            for w in range(W):
                k = [ld(i, r - DIL * w) for i in (4, 5, 6, 7, 13)]
                sw = (q[0] * k[0] + q[1] * k[1]) + (q[2] * k[2] + q[3] * k[3]) + q[4] * k[4]
                sw = sw + pltpu.roll(sw, 64, 1)
                sw = sw + pltpu.roll(sw, 32, 1)
                if 8 * j < DIL * w:
                    sw = jnp.where(sub8 + (t * T + 8 * j - DIL * w) >= 0, sw, NEG)
                s.append(sw)
            mx = functools.reduce(jnp.maximum, s)
            e = [jnp.exp2(sw - mx) for sw in s]
            rinv = pl.reciprocal(functools.reduce(lambda a, b: a + b, e), approx=True)
            o = None
            for oi, i in enumerate((8, 9, 10, 11, 12)):
                pv = (e[0] if o is None else _gate_f(e[0], token(o))) * ld(i, r)
                for w in range(1, W):
                    pv = pv + e[w] * ld(i, r - DIL * w)
                o = pv * rinv
                o_s[pl.ds(8 * j, 8), pl.ds(128 * oi, 128)] = o
            return token(o)

        z = None
        for j in range(T // 8):
            z = attn_rows(j, z)

        acc = acc_s[:, tile(t)]
        for c in range(len(CHUNKS)):
            a = acts[c] if c < NPRE else ffn1(xnb, bounds[c], bounds[c + 1])
            acc = acc + ffn2(a, bounds[c], bounds[c + 1])
        ob = o_s[...].astype(bf16)
        wop = wop_s[...]
        for n in range(NB):
            cs = cols(t * T + 128 * n, 128)
            fin = (acc[:, 128 * n:128 * (n + 1)] + jax.lax.dot_general(
                wop, ob[128 * n:128 * (n + 1)], NT, preferred_element_type=f32)).astype(bf16)
            for r0, r1, cp in out_copies(t, n):
                out_v[r0:r1, cs] = fin[r0:r1]
                cp.start()
        return carry

    jax.lax.fori_loop(0, NTILE, p2_body, 0)
    for t in range(NTILE):
        for n in range(NB):
            for _, _, cp in out_copies(t, n):
                cp.wait()


@jax.jit
def pallas_parallel_sum__sliding_local_dilated__dense_activation_mish__prompt_kernel(
    A_x: jax.Array,
    A_wqkv: jax.Array,
    A_wo: jax.Array,
    B_x: jax.Array,
    B_w1: jax.Array,
    B_b1: jax.Array,
    B_w2: jax.Array,
):
    del B_x
    hbm = pl.BlockSpec(memory_space=pl.ANY)
    out_t = pl.pallas_call(
        _kernel,
        in_specs=[hbm] * 6,
        out_specs=hbm,
        out_shape=jax.ShapeDtypeStruct((D, S), bf16),
        scratch_shapes=[
            pltpu.VMEM((D, S), bf16),
            pltpu.VMEM((D, 3 * D), bf16),
            pltpu.VMEM((D, D), bf16),
            pltpu.VMEM((D, F), bf16),
            pltpu.VMEM((F // 128, 128), bf16),
            pltpu.VMEM((D, F), bf16),
            pltpu.VMEM((S, D), bf16),
            pltpu.VMEM((D, S), f32),
            pltpu.VMEM((T, F0), bf16),
            pltpu.VMEM((3, 5, 640, 128), f32),
            pltpu.VMEM((3 * D, D), bf16),
            pltpu.VMEM((5, D, 128), f32),
            pltpu.VMEM((D, 640), bf16),
            pltpu.VMEM((14, HALO + T, 128), f32),
            pltpu.VMEM((T, 640), f32),
            pltpu.VMEM((D, S), bf16),
            pltpu.SMEM((1,), i32),
            pltpu.SemaphoreType.DMA((8 + NTILE,)),
            pltpu.SemaphoreType.DMA((NTILE * NOD,)),
        ],
        compiler_params=pltpu.CompilerParams(vmem_limit_bytes=100 * 1024 * 1024),
    )(A_x.reshape(S, D).T, A_wqkv, A_wo, B_w1, B_b1.reshape(F // 128, 128), B_w2.T)
    return out_t.T.reshape(1, S, D)
```

```python
import functools

import jax
import jax.numpy as jnp
import jax.experimental.pallas as pl
import jax.experimental.pallas.tpu as pltpu

S, D, F = 2048, 576, 4608
H, DH, W, DIL = 32, 18, 8, 2
T = 512
NTILE = S // T
NB = T // 128
HALO = 16
F0 = 768
FH = 256
CHUNKS = (768,) * 5
NPRE = 3
OSPLIT = (384, D)
NOD = NB - 1 + len(OSPLIT)
EPS = 1e-5
LOG2E = 1.4426950408889634
CEXP = DH ** -0.5 * LOG2E
NEG = -1e9 * LOG2E
f32, bf16, i32 = jnp.float32, jnp.bfloat16, jnp.int32
NT = (((1,), (1,)), ((), ()))


def _mish(h):
    u = jnp.exp(jnp.minimum(h, 20.0))
    n = u * (u + 2.0)
    return h * (n * pl.reciprocal(n + 2.0, approx=True))


def _gate(x, z, rows, dtype):
    if z is None:
        return x
    head = pltpu.bitcast(pltpu.bitcast(x[:rows, :128], i32) | z, dtype)
    if x.shape[1] > 128:
        head = jnp.concatenate([head, x[:rows, 128:]], axis=1)
    return jnp.concatenate([head, x[rows:]], axis=0) if x.shape[0] > rows else head


def _gate_f(x, z):
    return _gate(x, z, 8, f32)


def _gate_b(x, z):
    return _gate(x, z, 16, bf16)


def _wp_row(part, d):
    if d < 16:
        return part * 512 + d * 32
    return {0: 1536, 2: 1600, 1: 1664}[part] + (d - 16) * 32


def _gather_rows(s, start, width):
    parts = []
    for i in range(s.shape[0]):
        parts.append(s[i, pl.ds(start, H, stride=DH), :][:, :min(128, width - 128 * i)])
    return jnp.concatenate(parts, axis=1)


def _store_tiles(s, r0, val):
    for i in range(s.shape[0]):
        w = min(128, val.shape[1] - 128 * i)
        s[i, pl.ds(r0, val.shape[0]), :w] = val[:, 128 * i:128 * i + w]


def _prep_qkv(part, wqkv_v, wt_s, wp_s, zvec, z):
    lo = (part * D) // 128 * 128
    hi = min(-(-((part + 1) * D) // 128) * 128, 3 * D)
    for c0 in range(lo, hi, 128):
        cw = min(128, hi - c0)
        blk = wqkv_v[:, c0:c0 + cw]
        if cw == 128:
            blk = _gate_b(blk, z)
        wt = blk.T.astype(f32)
        _store_tiles(wt_s, c0 - lo, wt)
        z = pltpu.bitcast(wt[cw - 8:, 384:512], i32) & zvec
    for d in range(DH):
        rows = _gather_rows(wt_s, part * D - lo + d, D)
        if d % 3 == 0:
            rows = _gate_f(rows, z)
        rows = rows.astype(bf16)
        wp_s[pl.ds(_wp_row(part, d), H), :] = rows
        z = pltpu.bitcast(rows[:16, :128], i32) & zvec
    return z


def _prep_wo(wo_v, wof_s, wop_s, zvec):
    _store_tiles(wof_s, 0, wo_v[...].astype(f32))
    pieces = [_gather_rows(wof_s, d, D).astype(bf16) for d in range(16)]
    pieces.append(jnp.zeros((64, D), bf16))
    pieces += [_gather_rows(wof_s, d, D).astype(bf16) for d in (16, 17)]
    wopt = jnp.concatenate(pieces, axis=0).T
    wop_s[...] = wopt
    return (pltpu.bitcast(wopt[D - 16:, 512:], i32) | pltpu.bitcast(wopt[D - 16:, :128], i32)) & zvec


def _kernel(xt_hbm, wqkv_hbm, wo_hbm, w1_hbm, b1_hbm, w2t_hbm, out_hbm,
            x_v, wqkv_v, wo_v, w1_v, b1_v, w2_v, xn_s, acc_s, a_s, wt_s, wp_s, wof_s, wop_s,
            qkv_s, o_s, out_v, z_s, sem_in, sem_out):
    def cols(start, size):
        if isinstance(start, int):
            return pl.ds(start, size)
        return pl.ds(pl.multiple_of(start, 128), size)

    def tile(t):
        return cols(t * T, T)

    def cx(t):
        return pltpu.make_async_copy(xt_hbm.at[:, tile(t)], x_v.at[:, tile(t)], sem_in.at[8 + t])

    def cw(src, dst, lo, hi, k):
        return pltpu.make_async_copy(src.at[:, pl.ds(lo, hi - lo)], dst.at[:, pl.ds(lo, hi - lo)], sem_in.at[k])

    def out_copies(t, n):
        cs = cols(t * T + 128 * n, 128)
        if n < NB - 1:
            return [(0, D, pltpu.make_async_copy(out_v.at[:, cs], out_hbm.at[:, cs], sem_out.at[t * NOD + n]))]
        res, r0 = [], 0
        for k, r1 in enumerate(OSPLIT):
            res.append((r0, r1, pltpu.make_async_copy(out_v.at[r0:r1, cs], out_hbm.at[r0:r1, cs],
                                                      sem_out.at[t * NOD + n + k])))
            r0 = r1
        return res

    cb = pltpu.make_async_copy(b1_hbm, b1_v, sem_in.at[0])
    c1a = cw(w1_hbm, w1_v, 0, FH, 1)
    c1b = cw(w1_hbm, w1_v, FH, F0, 2)
    c2a = cw(w2t_hbm, w2_v, 0, F0, 3)
    cq = pltpu.make_async_copy(wqkv_hbm, wqkv_v, sem_in.at[4])
    co = pltpu.make_async_copy(wo_hbm, wo_v, sem_in.at[5])
    c1r = cw(w1_hbm, w1_v, F0, F, 6)
    c2r = cw(w2t_hbm, w2_v, F0, F, 7)
    for c in [cx(0), c1a, cb, c1b, c2a] + [cx(t) for t in range(1, NTILE)] + [cq, co, c1r, c2r]:
        c.start()

    z_s[0] = 0
    for i in range(4, 13):
        qkv_s[i, pl.ds(T, HALO), :] = jnp.zeros((HALO, 128), f32)
    qkv_s[13] = jnp.zeros((HALO + T, 128), f32)
    for part in range(3):
        wt_s[part, 4] = jnp.zeros(wt_s.shape[2:], f32)
    wof_s[4] = jnp.zeros(wof_s.shape[1:], f32)

    def zeros_vec():
        return jnp.full((8, 128), z_s[0], i32)

    def layernorm(start, ntok, blk):
        z = None
        for b in range(ntok // blk):
            sl = cols(start + blk * b, blk)
            xt = _gate_f(x_v[:, sl].astype(f32), z)
            xc = xt - jnp.mean(xt, axis=0, keepdims=True)
            v = jnp.mean(xc * xc, axis=0, keepdims=True)
            xn = (xc * jax.lax.rsqrt(v + EPS)).astype(bf16).T
            xn_s[sl, :] = xn
            z = (pltpu.bitcast(xn[blk - 16:, 384:512], i32) | pltpu.bitcast(xn[blk - 16:, :128], i32)) & zeros_vec()

    def bias(lo, hi):
        return jnp.concatenate([b1_v[pl.ds(i, 1), :] for i in range(lo // 128, hi // 128)], axis=1).astype(f32)

    def ffn1(xnb, lo, hi):
        return _mish(jnp.dot(xnb, w1_v[:, lo:hi], preferred_element_type=f32) + bias(lo, hi)).astype(bf16)

    def ffn1k(xnb, lo, hi, msplit):
        xa, xr = xnb[:, :512], xnb[:, 512:]
        mb = xnb.shape[0] // msplit
        rem = jnp.concatenate([jnp.dot(xr[i * mb:(i + 1) * mb], w1_v[512:, lo:hi], preferred_element_type=f32)
                               for i in range(msplit)], axis=0)
        outs = []
        for c0 in range(lo, hi, 128):
            h = jnp.dot(xa, w1_v[:512, c0:c0 + 128], preferred_element_type=f32)
            outs.append(_mish(h + (rem[:, c0 - lo:c0 - lo + 128] + bias(c0, c0 + 128))))
        return jnp.concatenate(outs, axis=1).astype(bf16)

    def ffn2(a, lo, hi):
        return jax.lax.dot_general(w2_v[:, lo:hi], a, NT, preferred_element_type=f32)

    def ffn2_first(t):
        w2c = w2_v[:, :F0]
        for n in range(NB):
            cs = cols(t * T + 128 * n, 128)
            acc_s[:, cs] = x_v[:, cs].astype(f32) + jax.lax.dot_general(
                w2c, a_s[128 * n:128 * (n + 1), :], NT, preferred_element_type=f32)

    HT = T // 2
    cx(0).wait()
    layernorm(0, HT, HT)
    c1a.wait()
    cb.wait()
    layernorm(HT, HT, HT)
    a_s[:HT, :FH] = ffn1k(xn_s[pl.ds(0, HT), :], 0, FH, 2)
    a_s[HT:, :FH] = ffn1k(xn_s[pl.ds(HT, HT), :], 0, FH, 2)
    c1b.wait()
    a_s[:, FH:] = ffn1k(xn_s[tile(0), :], FH, F0, 1)

    def p1_body(t, carry):
        @pl.when(t == 0)
        def _():
            c2a.wait()
        cx(t + 1).wait()
        layernorm((t + 1) * T, T, 128)
        ffn2_first(t)
        a_s[...] = ffn1k(xn_s[tile(t + 1), :], 0, F0, 2)
        return carry

    jax.lax.fori_loop(0, NTILE - 1, p1_body, 0)

    cq.wait()
    co.wait()
    zv = zeros_vec()
    z = _prep_wo(wo_v, wof_s, wop_s, zv)
    for part in range(3):
        z = _prep_qkv(part, wqkv_v, wt_s.at[part], wp_s, zv, z)
    ffn2_first(NTILE - 1)
    c1r.wait()
    c2r.wait()

    sub8 = jax.lax.broadcasted_iota(i32, (8, 128), 0)
    cexp_bits = pltpu.bitcast(jnp.full((8, 128), CEXP, f32), i32)

    def p2_body(t, carry):
        zvec = zeros_vec()
        xnb = xn_s[tile(t), :]
        bounds = [F0]
        for c in CHUNKS:
            bounds.append(bounds[-1] + c)
        acts = [ffn1k(xnb, bounds[0], bounds[1], 2)]
        acts += [ffn1(xnb, bounds[c], bounds[c + 1]) for c in range(1, NPRE)]

        for i in range(4, 14):
            qkv_s[i, pl.ds(0, HALO), :] = qkv_s[i, pl.ds(T, HALO), :]
        rem = jax.lax.dot_general(wp_s[pl.ds(1536, 192), :], xnb, NT, preferred_element_type=f32).T
        qkv_s[12, pl.ds(HALO, T), :] = rem[:, :128]
        qkv_s[13, pl.ds(HALO, T), :64] = rem[:, 128:]
        qkv = jax.lax.dot_general(xnb, wp_s[pl.ds(0, 1536), :], NT, preferred_element_type=f32)
        for i in range(12):
            qkv_s[i, pl.ds(HALO, T), :] = qkv[:, 128 * i:128 * (i + 1)]

        def ld(i, r):
            return qkv_s[i, pl.ds(r, 8), :]

        def token(x):
            return pltpu.bitcast(x, i32) & zvec

        def attn_rows(j, z):
            r = HALO + 8 * j
            scale = pltpu.bitcast(cexp_bits if z is None else cexp_bits | z, f32)
            q = [ld(i, r) * scale for i in (0, 1, 2, 3, 12)]
            s = []
            for w in range(W):
                k = [ld(i, r - DIL * w) for i in (4, 5, 6, 7, 13)]
                sw = (q[0] * k[0] + q[1] * k[1]) + (q[2] * k[2] + q[3] * k[3]) + q[4] * k[4]
                sw = sw + pltpu.roll(sw, 64, 1)
                sw = sw + pltpu.roll(sw, 32, 1)
                if 8 * j < DIL * w:
                    sw = jnp.where(sub8 + (t * T + 8 * j - DIL * w) >= 0, sw, NEG)
                s.append(sw)
            mx = functools.reduce(jnp.maximum, s)
            e = [jnp.exp2(sw - mx) for sw in s]
            rinv = pl.reciprocal(functools.reduce(lambda a, b: a + b, e), approx=True)
            o = None
            for oi, i in enumerate((8, 9, 10, 11, 12)):
                pv = (e[0] if o is None else _gate_f(e[0], token(o))) * ld(i, r)
                for w in range(1, W):
                    pv = pv + e[w] * ld(i, r - DIL * w)
                o = pv * rinv
                o_s[pl.ds(8 * j, 8), pl.ds(128 * oi, 128)] = o
            return token(o)

        z = None
        for j in range(T // 8):
            z = attn_rows(j, z)

        acc = acc_s[:, tile(t)]
        for c in range(len(CHUNKS)):
            a = acts[c] if c < NPRE else ffn1(xnb, bounds[c], bounds[c + 1])
            acc = acc + ffn2(a, bounds[c], bounds[c + 1])
        ob = o_s[...].astype(bf16)
        wop = wop_s[...]
        for n in range(NB):
            cs = cols(t * T + 128 * n, 128)
            fin = (acc[:, 128 * n:128 * (n + 1)] + jax.lax.dot_general(
                wop, ob[128 * n:128 * (n + 1)], NT, preferred_element_type=f32)).astype(bf16)
            for r0, r1, cp in out_copies(t, n):
                out_v[r0:r1, cs] = fin[r0:r1]
                cp.start()
        return carry

    jax.lax.fori_loop(0, NTILE, p2_body, 0)
    for t in range(NTILE):
        for n in range(NB):
            for _, _, cp in out_copies(t, n):
                cp.wait()


@jax.jit
def pallas_parallel_sum__sliding_local_dilated__dense_activation_mish__prompt_kernel(
    A_x: jax.Array,
    A_wqkv: jax.Array,
    A_wo: jax.Array,
    B_x: jax.Array,
    B_w1: jax.Array,
    B_b1: jax.Array,
    B_w2: jax.Array,
):
    del B_x
    hbm = pl.BlockSpec(memory_space=pl.ANY)
    out_t = pl.pallas_call(
        _kernel,
        in_specs=[hbm] * 6,
        out_specs=hbm,
        out_shape=jax.ShapeDtypeStruct((D, S), bf16),
        scratch_shapes=[
            pltpu.VMEM((D, S), bf16),
            pltpu.VMEM((D, 3 * D), bf16),
            pltpu.VMEM((D, D), bf16),
            pltpu.VMEM((D, F), bf16),
            pltpu.VMEM((F // 128, 128), bf16),
            pltpu.VMEM((D, F), bf16),
            pltpu.VMEM((S, D), bf16),
            pltpu.VMEM((D, S), f32),
            pltpu.VMEM((T, F0), bf16),
            pltpu.VMEM((3, 5, 640, 128), f32),
            pltpu.VMEM((3 * D, D), bf16),
            pltpu.VMEM((5, D, 128), f32),
            pltpu.VMEM((D, 640), bf16),
            pltpu.VMEM((14, HALO + T, 128), f32),
            pltpu.VMEM((T, 640), f32),
            pltpu.VMEM((D, S), bf16),
            pltpu.SMEM((1,), i32),
            pltpu.SemaphoreType.DMA((8 + NTILE,)),
            pltpu.SemaphoreType.DMA((NTILE * NOD,)),
        ],
        compiler_params=pltpu.CompilerParams(vmem_limit_bytes=100 * 1024 * 1024),
    )(A_x.reshape(S, D).T, A_wqkv, A_wo, B_w1, B_b1.reshape(F // 128, 128), B_w2.T)
    return out_t.T.reshape(1, S, D)
```

```python
import functools

import jax
import jax.numpy as jnp
import jax.experimental.pallas as pl
import jax.experimental.pallas.tpu as pltpu

S, D, F = 2048, 576, 4608
H, DH, W, DIL = 32, 18, 8, 2
T = 512
NTILE = S // T
NB = T // 128
HALO = 16
F0 = 768
FH = 256
FX = 256
F1 = F0 + FX
CHUNKS = (3584,)
NPRE = 1
HT = T // 2
HD = D // 2
PACE = 1
PR = 16
PIPE = 1
ROT3 = 1
QSPLIT = 2
QS = 1
QROLL = 1
QH = 0
NPX = 2
GR = 128
GD_ = 128
LAG = 1
PB = 8
NPC = 2
HOPS = 3
ONECH = 1
PROWS = (HT - 8,)
OSPLIT = (384, D)
NOD = NB - 1 + len(OSPLIT)
EPS = 1e-5
LOG2E = 1.4426950408889634
CEXP = DH ** -0.5 * LOG2E
NEG = -1e9 * LOG2E
f32, bf16, i32 = jnp.float32, jnp.bfloat16, jnp.int32


def _pk(x):
    return pltpu.bitcast(x, i32)


def _un(x):
    return pltpu.bitcast(x, bf16)


def _even_odd(x):
    w = pltpu.bitcast(x, jnp.uint32)
    return tuple(pltpu.unpack_elementwise(w, index=k, packed_dtype=bf16, unpacked_dtype=f32) for k in range(2))


def _zip_rows(e, o):
    return pltpu.bitcast(pltpu.pack_elementwise([e, o], packed_dtype=bf16), i32)

NT = (((1,), (1,)), ((), ()))


def _mish(h):
    u = jnp.exp(jnp.minimum(h, 20.0))
    n = u * (u + 2.0)
    return h * (n * pl.reciprocal(n + 2.0, approx=True))


def _gate(x, z, rows, dtype):
    if z is None:
        return x
    head = pltpu.bitcast(pltpu.bitcast(x[:rows, :128], i32) | z, dtype)
    if x.shape[1] > 128:
        head = jnp.concatenate([head, x[:rows, 128:]], axis=1)
    return jnp.concatenate([head, x[rows:]], axis=0) if x.shape[0] > rows else head


def _gate_f(x, z):
    return _gate(x, z, 8, f32)


def _gate_b(x, z):
    return _gate(x, z, 16, bf16)


def _wp_row(part, d):
    if d < 16:
        return part * 512 + d * 32
    return {0: 1536, 2: 1600, 1: 1664}[part] + (d - 16) * 32


def _gather_rows(s, start, width):
    parts = []
    for i in range(s.shape[0]):
        parts.append(s[i, pl.ds(start, H, stride=DH), :][:, :min(128, width - 128 * i)])
    return jnp.concatenate(parts, axis=1)


def _store_tiles(s, r0, val):
    for i in range(s.shape[0]):
        w = min(128, val.shape[1] - 128 * i)
        s[i, pl.ds(r0, val.shape[0]), :w] = val[:, 128 * i:128 * i + w]


def _prep_qkv(part, wqkv_v, wt_s, wp_s, zvec, z):
    lo = (part * D) // 128 * 128
    hi = min(-(-((part + 1) * D) // 128) * 128, 3 * D)
    for c0 in range(lo, hi, 128):
        cw = min(128, hi - c0)
        blk = wqkv_v[:, c0:c0 + cw]
        if cw == 128:
            blk = _gate_b(blk, z)
        wt = blk.T.astype(f32)
        _store_tiles(wt_s, c0 - lo, wt)
        z = pltpu.bitcast(wt[cw - 8:, 384:512], i32) & zvec
    for d in range(DH):
        rows = _gather_rows(wt_s, part * D - lo + d, D)
        if d % 3 == 0:
            rows = _gate_f(rows, z)
        rows = rows.astype(bf16)
        wp_s[pl.ds(_wp_row(part, d) // 2, H // 2), :] = _pk(rows)
        z = pltpu.bitcast(rows[:16, :128], i32) & zvec
    return z


def _prep_wo(wo_v, wof_s, wop_s, zvec):
    _store_tiles(wof_s, 0, wo_v[...].astype(f32))
    pieces = [_gather_rows(wof_s, d, D).astype(bf16) for d in range(16)]
    pieces.append(jnp.zeros((64, D), bf16))
    pieces += [_gather_rows(wof_s, d, D).astype(bf16) for d in (16, 17)]
    wopt = jnp.concatenate(pieces, axis=0).T
    wop_s[...] = _pk(wopt)
    return (pltpu.bitcast(wopt[D - 16:, 512:], i32) | pltpu.bitcast(wopt[D - 16:, :128], i32)) & zvec


def _kernel(xt_hbm, wqkv_hbm, wo_hbm, w1_hbm, b1_hbm, w2t_hbm, out_hbm,
            x_v, wqkv_v, wo_v, w1_v, b1_v, w2_v, xn_s, acc_s, a_s, wt_s, wp_s, wof_s, wop_s,
            qkv_s, o_s, out_v, s1_s, s2_s, sq_s, z_s, sem_in, sem_out):
    def cols(start, size):
        if isinstance(start, int):
            return pl.ds(start, size)
        return pl.ds(pl.multiple_of(start, 128), size)

    def tile(t):
        return cols(t * T, T)

    def prows(start, size):
        if isinstance(start, int):
            return pl.ds(start // 2, size // 2)
        return pl.ds(pl.multiple_of(start // 2, 64), size // 2)

    def xn_at(start, size):
        return _un(xn_s[prows(start, size), :])

    def cx(t):
        return pltpu.make_async_copy(xt_hbm.at[:, tile(t)], x_v.at[:, tile(t)], sem_in.at[8 + t])

    def cw(src, dst, lo, hi, k):
        return pltpu.make_async_copy(src.at[:, pl.ds(lo, hi - lo)], dst.at[:, pl.ds(lo, hi - lo)], sem_in.at[k])

    def out_copies(t, n):
        cs = cols(t * T + 128 * n, 128)
        if n < NB - 1:
            return [(0, D, pltpu.make_async_copy(out_v.at[:, cs], out_hbm.at[:, cs], sem_out.at[t * NOD + n]))]
        res, r0 = [], 0
        for k, r1 in enumerate(OSPLIT):
            res.append((r0, r1, pltpu.make_async_copy(out_v.at[r0:r1, cs], out_hbm.at[r0:r1, cs],
                                                      sem_out.at[t * NOD + n + k])))
            r0 = r1
        return res

    cb = pltpu.make_async_copy(b1_hbm, b1_v, sem_in.at[0])
    c1a = cw(w1_hbm, w1_v, 0, FH, 1)
    c1b = cw(w1_hbm, w1_v, FH, F0, 2)
    c2a = cw(w2t_hbm, w2_v, 0, F0, 3)
    cq = pltpu.make_async_copy(wqkv_hbm, wqkv_v, sem_in.at[4])
    co = pltpu.make_async_copy(wo_hbm, wo_v, sem_in.at[5])
    c1r = cw(w1_hbm, w1_v, F0, F, 6)
    c2r = cw(w2t_hbm, w2_v, F0, F, 7)
    bounds = [F1]
    for c in CHUNKS:
        bounds.append(bounds[-1] + c)
    assert bounds[-1] == F
    for c in [cx(0), c1a, cb, c1b, c2a] + [cx(t) for t in range(1, NTILE)] + [cq, co, c1r, c2r]:
        c.start()

    z_s[0] = 0
    for i in range(4, 13):
        qkv_s[i, pl.ds(T, HALO), :] = jnp.zeros((HALO, 128), f32)
    qkv_s[13] = jnp.zeros((HALO + T, 128), f32)
    for part in range(3):
        wt_s[part, 4] = jnp.zeros(wt_s.shape[2:], f32)
    wof_s[4] = jnp.zeros(wof_s.shape[1:], f32)

    def zeros_vec():
        return jnp.full((8, 128), z_s[0], i32)

    def layernorm(start, ntok, blk):
        z = None
        for b in range(ntok // blk):
            sl = cols(start + blk * b, blk)
            xt = _gate_f(x_v[:, sl].astype(f32), z)
            xc = xt - jnp.mean(xt, axis=0, keepdims=True)
            v = jnp.mean(xc * xc, axis=0, keepdims=True)
            xn = (xc * jax.lax.rsqrt(v + EPS)).astype(bf16).T
            xn_s[prows(start + blk * b, blk), :] = _pk(xn)
            z = (pltpu.bitcast(xn[blk - 16:, 384:512], i32) | pltpu.bitcast(xn[blk - 16:, :128], i32)) & zeros_vec()

    def bias(lo, hi):
        return jnp.concatenate([b1_v[pl.ds(i, 1), :] for i in range(lo // 128, hi // 128)], axis=1).astype(f32)

    def ffn1(xnb, lo, hi):
        return _mish(jnp.dot(xnb, w1_v[:, lo:hi], preferred_element_type=f32) + bias(lo, hi)).astype(bf16)

    def ffn1k(xnb, lo, hi, msplit):
        xa, xr = xnb[:, :512], xnb[:, 512:]
        mb = xnb.shape[0] // msplit
        rem = jnp.concatenate([jnp.dot(xr[i * mb:(i + 1) * mb], w1_v[512:, lo:hi], preferred_element_type=f32)
                               for i in range(msplit)], axis=0)
        outs = []
        for c0 in range(lo, hi, 128):
            h = jnp.dot(xa, w1_v[:512, c0:c0 + 128], preferred_element_type=f32)
            outs.append(_mish(h + (rem[:, c0 - lo:c0 - lo + 128] + bias(c0, c0 + 128))))
        return jnp.concatenate(outs, axis=1).astype(bf16)

    def ffn2(a, lo, hi):
        return jax.lax.dot_general(w2_v[:, lo:hi], a, NT, preferred_element_type=f32)

    def ffn2_first(t):
        w2c = w2_v[:, :F0]
        for n in range(NB):
            cs = cols(t * T + 128 * n, 128)
            acc_s[:, cs] = x_v[:, cs].astype(f32) + jax.lax.dot_general(
                w2c, _un(a_s[64 * n:64 * (n + 1), :]), NT, preferred_element_type=f32)

    cx(0).wait()
    layernorm(0, HT, HT)
    c1a.wait()
    cb.wait()
    layernorm(HT, HT, HT)
    a_s[:HT // 2, :FH] = _pk(ffn1k(xn_at(0, HT), 0, FH, 2))
    a_s[HT // 2:, :FH] = _pk(ffn1k(xn_at(HT, HT), 0, FH, 2))
    c1b.wait()
    a_s[:, FH:] = _pk(ffn1k(xn_at(0, T), FH, F0, 1))

    def p1_body(t, carry):
        @pl.when(t == 0)
        def _():
            c2a.wait()
        cx(t + 1).wait()
        layernorm((t + 1) * T, T, 128)
        ffn2_first(t)
        a_s[...] = _pk(ffn1k(xn_at((t + 1) * T, T), 0, F0, 2))
        return carry

    jax.lax.fori_loop(0, NTILE - 1, p1_body, 0)

    cq.wait()
    co.wait()
    zv = zeros_vec()
    z = _prep_wo(wo_v, wof_s, wop_s, zv)
    for part in range(3):
        z = _prep_qkv(part, wqkv_v, wt_s.at[part], wp_s, zv, z)
    ffn2_first(NTILE - 1)
    c1r.wait()
    c2r.wait()

    up = lambda v: v.astype(f32)
    def px_body(it, carry):
        zs = [None, None]
        for c in range(len(CHUNKS)):
            half = CHUNKS[c] // 2
            for g0 in range(0, half, 256):
                lc, rc, sj = bounds[c] + g0, bounds[c] + half + g0, (bounds[c] - F1) // 2 + g0
                for k, (w_v, s_s, hr) in enumerate(((w1_v, s1_s, 256), (w2_v, s2_s, HD))):
                    for r1 in range(0, hr // NPX, PR):
                        r0 = it * (hr // NPX) + r1
                        blk = [_even_odd(w_v[pl.ds(pl.multiple_of(ro + r0, 16), PR), co:co + 256])
                               for ro in (0, hr) for co in (lc, rc)]
                        sums = []
                        for par in range(2):
                            p11, p12, p21, p22 = [b[par] for b in blk]
                            if zs[k] is not None:
                                zf = jnp.tile(zs[k], (PR // 16, 2))
                                p11 = pltpu.bitcast(pltpu.bitcast(p11, i32) | zf, f32)
                                p22 = pltpu.bitcast(pltpu.bitcast(p22, i32) | zf, f32)
                            if k == 0:
                                sums.append((p11 + p22, p12 - p22, p21 - p11, p11 + p12, p21 + p22))
                            else:
                                sums.append((p11 + p22, p21 + p22, p11 + p12, p21 - p11, p12 - p22))
                        for n in range(5):
                            v = _zip_rows(sums[0][n], sums[1][n])
                            s_s[n, pl.ds(pl.multiple_of(r0 // 2, 8), PR // 2), sj:sj + 256] = v
                        zn = v[PR // 2 - 8:, 128:] & zv
                        for _ in range(HOPS):
                            zn = pltpu.bitcast(jnp.exp2(pltpu.bitcast(zn, f32)), i32) & zv
                        zs[0] = zs[1] = zn
        zq = None
        if QS:
            for r1 in range(0, 768 // NPX, PR):
                r0 = it * (768 // NPX) + r1
                blk = [_even_odd(_un(wp_s[pl.ds(pl.multiple_of((ro + r0) // 2, 8), PR // 2), co:co + 256]))
                       for co in (0, 256) for ro in (0, 768)]
                sums = []
                for par in range(2):
                    p11, p12, p21, p22 = [b[par] for b in blk]
                    if zq is not None:
                        zf = jnp.tile(zq, (PR // 16, 2))
                        p11 = pltpu.bitcast(pltpu.bitcast(p11, i32) | zf, f32)
                        p22 = pltpu.bitcast(pltpu.bitcast(p22, i32) | zf, f32)
                    sums.append((p11 + p22, p12 - p22, p21 - p11, p11 + p12, p21 + p22))
                for n in range(5):
                    v = _zip_rows(sums[0][n], sums[1][n])
                    sq_s[n, pl.ds(pl.multiple_of(r0 // 2, 8), PR // 2), :] = v
                zq = pltpu.roll(v[PR // 2 - 8:, 128:] & zv, QROLL, 1)
                for _ in range(QH):
                    zq = pltpu.roll(zq, QROLL, 1)
        nt = NTILE // NPX
        ax = [ffn1(xn_at((it * nt + t) * T, T), F0, F1) for t in range(nt)]
        for t in range(nt):
            acc_s[:, tile(it * nt + t)] = acc_s[:, tile(it * nt + t)] + ffn2(ax[t], F0, F1)
        return carry

    jax.lax.fori_loop(0, NPX, px_body, 0)

    sub8 = jax.lax.broadcasted_iota(i32, (8, 128), 0)
    cexp_bits = pltpu.bitcast(jnp.full((8, 128), CEXP, f32), i32)

    def p2_body(t, carry):
        zvec = zeros_vec()
        xnb = xn_at(t * T, T)
        dot = lambda a, b: jnp.dot(a, b, preferred_element_type=f32)
        xe, xo = _even_odd(xnb)
        xf = jnp.concatenate([xe[:HT // 2], xo[:HT // 2], xe[HT // 2:], xo[HT // 2:]], axis=0)
        f11, f12, f21, f22 = xf[:HT, :256], xf[:HT, 256:512], xf[HT:, :256], xf[HT:, 256:512]
        x11, x22, xr = f11.astype(bf16), f22.astype(bf16), xf[:, 512:].astype(bf16)
        xs = [v.astype(bf16) for v in (f11 + f22, f21 + f22, f11 + f12, f21 - f11, f12 - f22)]
        pace = [None, None]

        def s_dots(c, g0):
            half = CHUNKS[c] // 2
            lc, rc, sj = bounds[c] + g0, bounds[c] + half + g0, (bounds[c] - F1) // 2 + g0
            sw = lambda n: _un(s1_s[n, :, sj:sj + GD_])
            rr = dot(xr, w1_v[512:, rc:rc + GD_])
            rl = dot(xr, w1_v[512:, lc:lc + GD_])
            m3 = dot(x11, sw(1))
            m5 = dot(xs[2], w1_v[256:512, rc:rc + GD_])
            m4 = dot(x22, sw(2))
            m2 = dot(xs[1], w1_v[:256, lc:lc + GD_])
            m1 = dot(xs[0], sw(0))
            m7 = dot(xs[4], sw(4))
            m6 = dot(xs[3], sw(3))
            return (rl[:HT], rl[HT:], rr[:HT], rr[HT:], m1, m2, m3, m4, m5, m6, m7), (lc, rc)

        ptok = [None] * NPC
        cnt = [0]

        def s_post(ms):
            ms, (lc, rc) = ms
            bl = jnp.broadcast_to(bias(lc, lc + 128), (8, 128))
            br = jnp.broadcast_to(bias(rc, rc + 128), (8, 128))
            outs = []
            for r0 in range(0, HT // 2, PB):
                ch = cnt[0] % NPC
                cnt[0] += 1
                o = []
                for rr0 in (r0, HT // 2 + r0):
                    blg = jnp.tile(_gate_f(bl, ptok[ch]), (PB // 8, 1))
                    brg = jnp.tile(_gate_f(br, ptok[ch]), (PB // 8, 1))
                    rlt, rlb, rrt, rrb, m1, m2, m3, m4, m5, m6, m7 = [v[rr0:rr0 + PB] for v in ms]
                    a12 = _mish((m3 + m5) + (rrt + brg))
                    a21 = _mish((m2 + m4) + (rlb + blg))
                    a11 = _mish((m1 + m4) + (m7 - m5) + (rlt + blg))
                    a22 = _mish((m1 - m2) + (m3 + m6) + (rrb + brg))
                    o.append((a11 + a22, a11, a21 - a22, a12 - a11, a22, a11 + a21, a12 + a22))
                    if rr0 == r0:
                        ptok[ch] = pltpu.bitcast(o[0][5][PB - 8:] + o[0][6][PB - 8:], i32) & zvec
                w = [_zip_rows(o[0][n], o[1][n]) for n in range(7)]
                outs.append(w)
                ptok[ch] = functools.reduce(lambda a, b: a | b, [v[PB - 8:] for v in w]) & zvec
            return [jnp.concatenate([o[n] for o in outs], axis=0) for n in range(7)]

        pend = []
        done = {}

        def flush_one():
            c, g0, ms = pend.pop(0)
            done.setdefault(c, []).append(s_post(ms))

        def sffn1(c):
            for g0 in range(0, CHUNKS[c] // 2, GD_):
                pend.append((c, g0, s_dots(c, g0)))
                if len(pend) > LAG:
                    flush_one()

        def sffn2(c, ms):
            half, lo, sj = CHUNKS[c] // 2, bounds[c], (bounds[c] - F1) // 2
            sw = lambda n: _un(s2_s[n, :, sj:sj + half])
            lhs = (sw(0), sw(1), w2_v[:HD, lo:lo + half], w2_v[HD:, lo + half:lo + 2 * half], sw(2), sw(3), sw(4))
            out = []
            for n in range(7):
                p = jax.lax.dot_general(lhs[n], _un(jnp.concatenate([d[n] for d in done[c]], axis=1)), NT, preferred_element_type=f32)
                out.append(p if ms is None else ms[n] + p)
            return out

        for c in range(NPRE):
            sffn1(c)

        for i in range(4, 14):
            qkv_s[i, pl.ds(0, HALO), :] = qkv_s[i, pl.ds(T, HALO), :]
        for q0 in (range(0, T, T // QSPLIT) if not QS else ()):
            qn = T // QSPLIT
            xq = xnb[q0:q0 + qn]
            rem = jax.lax.dot_general(_un(wp_s[pl.ds(768, 96), :]), xq, NT, preferred_element_type=f32).T
            qkv_s[12, pl.ds(HALO + q0, qn), :] = rem[:, :128]
            qkv_s[13, pl.ds(HALO + q0, qn), :64] = rem[:, 128:]
            qkv = jax.lax.dot_general(xq, _un(wp_s[pl.ds(0, 768), :]), NT, preferred_element_type=f32)
            for i in range(12):
                qkv_s[i, pl.ds(HALO + q0, qn), :] = qkv[:, 128 * i:128 * (i + 1)]

        if QS:
            dt = lambda a, b: jax.lax.dot_general(a, b, NT, preferred_element_type=f32)
            rem = dt(_un(wp_s[pl.ds(768, 96), :]), xnb).T
            qkv_s[12, pl.ds(HALO, T), :] = rem[:, :128]
            qkv_s[13, pl.ds(HALO, T), :64] = rem[:, 128:]
            n11, n12, n21, n22 = xnb[:HT, :256], xnb[:HT, 256:512], xnb[HT:, :256], xnb[HT:, 256:512]
            ns = [(up(p) + sg * up(q)).astype(bf16) for p, q, sg in
                  ((n11, n22, 1.0), (n21, n22, 1.0), (n11, n12, 1.0), (n21, n11, -1.0), (n12, n22, -1.0))]
            nr = xnb[:, 512:]
            for i in range(6):
                wl = lambda lo, hi, i=i: _un(wp_s[pl.ds(64 * i, 64), lo:hi])
                wr = lambda lo, hi, i=i: _un(wp_s[pl.ds(384 + 64 * i, 64), lo:hi])
                sw = lambda n, i=i: _un(sq_s[n, pl.ds(64 * i, 64), :])
                rl, rr = dt(nr, wl(512, D)), dt(nr, wr(512, D))
                m3, m5 = dt(n11, sw(1)), dt(ns[2], wr(256, 512))
                m4, m2 = dt(n22, sw(2)), dt(ns[1], wl(0, 256))
                m1, m7, m6 = dt(ns[0], sw(0)), dt(ns[4], sw(4)), dt(ns[3], sw(3))
                qkv_s[6 + i, pl.ds(HALO, HT), :] = (m3 + m5) + rr[:HT]
                qkv_s[i, pl.ds(HALO + HT, HT), :] = (m2 + m4) + rl[HT:]
                qkv_s[i, pl.ds(HALO, HT), :] = (m1 + m4) + (m7 - m5) + rl[:HT]
                qkv_s[6 + i, pl.ds(HALO + HT, HT), :] = (m1 - m2) + (m3 + m6) + rr[HT:]

        while pend:
            flush_one()

        def ld(i, r):
            return qkv_s[i, pl.ds(r, 8), :]

        def token(x):
            return pltpu.bitcast(x, i32) & zvec

        def qk(j, z):
            r = HALO + 8 * j
            scale = pltpu.bitcast(cexp_bits if z is None else cexp_bits | z, f32)
            q = [ld(i, r) * scale for i in (0, 1, 2, 3, 12)]
            raw = []
            for w in range(W):
                k = [ld(i, r - DIL * w) for i in (4, 5, 6, 7, 13)]
                raw.append((q[0] * k[0] + q[1] * k[1]) + (q[2] * k[2] + q[3] * k[3]) + q[4] * k[4])
            return raw

        def softmax(j, raw):
            s = []
            for w, sw in enumerate(raw):
                if ROT3:
                    sw = (sw + pltpu.roll(sw, 64, 1)) + (pltpu.roll(sw, 32, 1) + pltpu.roll(sw, 96, 1))
                else:
                    sw = sw + pltpu.roll(sw, 64, 1)
                    sw = sw + pltpu.roll(sw, 32, 1)
                if 8 * j < DIL * w:
                    sw = jnp.where(sub8 + (t * T + 8 * j - DIL * w) >= 0, sw, NEG)
                s.append(sw)
            mx = functools.reduce(jnp.maximum, s)
            e = [jnp.exp2(sw - mx) for sw in s]
            rinv = pl.reciprocal(functools.reduce(lambda a, b: a + b, e), approx=True)
            return e, rinv

        def pv(j, e, rinv, z):
            r = HALO + 8 * j
            for oi, i in enumerate((8, 9, 10, 11, 12)):
                p = _gate_f(e[0], z) * ld(i, r)
                for w in range(1, W):
                    p = p + e[w] * ld(i, r - DIL * w)
                o = p * rinv
                o_s[pl.ds(8 * j, 8), pl.ds(128 * oi, 128)] = o
                z = token(o)
            return z

        if PIPE:
            raw = qk(0, None)
            for j in range(T // 8):
                e, rinv = softmax(j, raw)
                zq = None
                if j + 1 < T // 8:
                    raw = qk(j + 1, token(rinv))
                    zq = token(raw[W - 1])
                pv(j, e, rinv, zq)
        else:
            z = None
            for j in range(T // 8):
                e, rinv = softmax(j, qk(j, z))
                z = pv(j, e, rinv, None)

        ms = None
        emitted = set(range(NPRE))
        for c in range(len(CHUNKS)):
            if c + 1 >= NPRE and c + 1 < len(CHUNKS) and c + 1 >= NPRE and (c + 1) not in emitted:
                sffn1(c + 1)
                emitted.add(c + 1)
            ms = sffn2(c, ms)
            while pend:
                flush_one()
        m1, m2, m3, m4, m5, m6, m7 = ms
        acc = acc_s[:, tile(t)] + jnp.concatenate(
            [jnp.concatenate([(m1 + m4) + (m7 - m5), m3 + m5], axis=1),
             jnp.concatenate([m2 + m4, (m1 - m2) + (m3 + m6)], axis=1)], axis=0)
        ob = o_s[...].astype(bf16)
        wop = _un(wop_s[...])
        for n in range(NB):
            cs = cols(t * T + 128 * n, 128)
            fin = (acc[:, 128 * n:128 * (n + 1)] + jax.lax.dot_general(
                wop, ob[128 * n:128 * (n + 1)], NT, preferred_element_type=f32)).astype(bf16)
            for r0, r1, cp in out_copies(t, n):
                out_v[r0:r1, cs] = fin[r0:r1]
                cp.start()
        return carry

    jax.lax.fori_loop(0, NTILE, p2_body, 0)
    for t in range(NTILE):
        for n in range(NB):
            for _, _, cp in out_copies(t, n):
                cp.wait()


@jax.jit
def pallas_parallel_sum__sliding_local_dilated__dense_activation_mish__prompt_kernel(
    A_x: jax.Array,
    A_wqkv: jax.Array,
    A_wo: jax.Array,
    B_x: jax.Array,
    B_w1: jax.Array,
    B_b1: jax.Array,
    B_w2: jax.Array,
):
    del B_x
    hbm = pl.BlockSpec(memory_space=pl.ANY)
    out_t = pl.pallas_call(
        _kernel,
        in_specs=[hbm] * 6,
        out_specs=hbm,
        out_shape=jax.ShapeDtypeStruct((D, S), bf16),
        scratch_shapes=[
            pltpu.VMEM((D, S), bf16),
            pltpu.VMEM((D, 3 * D), bf16),
            pltpu.VMEM((D, D), bf16),
            pltpu.VMEM((D, F), bf16),
            pltpu.VMEM((F // 128, 128), bf16),
            pltpu.VMEM((D, F), bf16),
            pltpu.VMEM((S // 2, D), i32),
            pltpu.VMEM((D, S), f32),
            pltpu.VMEM((T // 2, F0), i32),
            pltpu.VMEM((3, 5, 640, 128), f32),
            pltpu.VMEM((3 * D // 2, D), i32),
            pltpu.VMEM((5, D, 128), f32),
            pltpu.VMEM((D // 2, 640), i32),
            pltpu.VMEM((14, HALO + T, 128), f32),
            pltpu.VMEM((T, 640), f32),
            pltpu.VMEM((D, S), bf16),
            pltpu.VMEM((5, 128, (F - F1) // 2), i32),
            pltpu.VMEM((5, HD // 2, (F - F1) // 2), i32),
            pltpu.VMEM((5, 384, 256), i32),
            pltpu.SMEM((1,), i32),
            pltpu.SemaphoreType.DMA((8 + NTILE,)),
            pltpu.SemaphoreType.DMA((NTILE * NOD,)),
        ],
        compiler_params=pltpu.CompilerParams(vmem_limit_bytes=100 * 1024 * 1024),
    )(A_x.reshape(S, D).T, A_wqkv, A_wo, B_w1, B_b1.reshape(F // 128, 128), B_w2.T)
    return out_t.T.reshape(1, S, D)
```

```python
import functools

import jax
import jax.numpy as jnp
import jax.experimental.pallas as pl
import jax.experimental.pallas.tpu as pltpu

S, D, F = 2048, 576, 4608
H, DH, W, DIL = 32, 18, 8, 2
T = 512
HT, HD = T // 2, D // 2
NTILE = S // T
NB = T // 128
HALO = 16
FH = 256
FA = 128
F0 = 384
F1 = 1024
FS = (F - F1) // 2
NG = FS // 128
NPX = 2
L2_ORDER = (2, 3, 6, 5, 0, 1, 4)
L2_PRE = (2, 3, 6, 5)
OSPLIT = (384, D)
NOD = NB - 1 + len(OSPLIT)
EPS = 1e-5
LOG2E = 1.4426950408889634
CEXP = DH ** -0.5 * LOG2E
NEG = -1e9 * LOG2E
f32, bf16, i32 = jnp.float32, jnp.bfloat16, jnp.int32
NT = (((1,), (1,)), ((), ()))


def _mo(v, n):
    return v if isinstance(v, int) else pl.multiple_of(v, n)


def _pk(x):
    return pltpu.bitcast(x, i32)


def _un(x):
    return pltpu.bitcast(x, bf16)


def _even_odd(x):
    w = pltpu.bitcast(x, jnp.uint32)
    return tuple(pltpu.unpack_elementwise(w, index=k, packed_dtype=bf16, unpacked_dtype=f32) for k in range(2))


def _zip_rows(e, o):
    return pltpu.bitcast(pltpu.pack_elementwise([e, o], packed_dtype=bf16), i32)


def _dot(a, b):
    return jnp.dot(a, b, preferred_element_type=f32)


def _dott(a, b):
    return jax.lax.dot_general(a, b, NT, preferred_element_type=f32)


def _sums_a(p11, p12, p21, p22):
    return p11 + p22, p21 + p22, p11 + p12, p21 - p11, p12 - p22


def _sums_b(p11, p12, p21, p22):
    return p11 + p22, p12 - p22, p21 - p11, p11 + p12, p21 + p22


def _combine(m1, m2, m3, m4, m5, m6, m7):
    return jnp.concatenate(
        [jnp.concatenate([(m1 + m4) + (m7 - m5), m3 + m5], axis=1),
         jnp.concatenate([m2 + m4, (m1 - m2) + (m3 + m6)], axis=1)], axis=0)


def _mish(h):
    u = jnp.exp(jnp.minimum(h, 20.0))
    n = u * (u + 2.0)
    return h * (n * pl.reciprocal(n + 2.0, approx=True))


def _gate(x, z, rows, dtype):
    if z is None:
        return x
    head = pltpu.bitcast(pltpu.bitcast(x[:rows, :128], i32) | z, dtype)
    if x.shape[1] > 128:
        head = jnp.concatenate([head, x[:rows, 128:]], axis=1)
    return jnp.concatenate([head, x[rows:]], axis=0) if x.shape[0] > rows else head


def _gate_f(x, z):
    return _gate(x, z, 8, f32)


def _gate_b(x, z):
    return _gate(x, z, 16, bf16)


def _wp_row(part, d):
    if d < 16:
        return part * 512 + d * 32
    return {0: 1536, 2: 1600, 1: 1664}[part] + (d - 16) * 32


def _gather_rows(s, start, width):
    parts = []
    for i in range(s.shape[0]):
        parts.append(s[i, pl.ds(start, H, stride=DH), :][:, :min(128, width - 128 * i)])
    return jnp.concatenate(parts, axis=1)


def _store_tiles(s, r0, val):
    for i in range(s.shape[0]):
        w = min(128, val.shape[1] - 128 * i)
        s[i, pl.ds(r0, val.shape[0]), :w] = val[:, 128 * i:128 * i + w]


def _prep_qkv(part, wqkv_v, wt_s, wp_s, zvec, z):
    lo = (part * D) // 128 * 128
    hi = min(-(-((part + 1) * D) // 128) * 128, 3 * D)
    for c0 in range(lo, hi, 128):
        cw = min(128, hi - c0)
        blk = wqkv_v[:, c0:c0 + cw]
        if cw == 128:
            blk = _gate_b(blk, z)
        wt = blk.T.astype(f32)
        _store_tiles(wt_s, c0 - lo, wt)
        z = pltpu.bitcast(wt[cw - 8:, 384:512], i32) & zvec
    for d in range(DH):
        rows = _gather_rows(wt_s, part * D - lo + d, D)
        if d % 3 == 0:
            rows = _gate_f(rows, z)
        rows = rows.astype(bf16)
        wp_s[pl.ds(_wp_row(part, d) // 2, H // 2), :] = _pk(rows)
        z = pltpu.bitcast(rows[:16, :128], i32) & zvec
    return z


def _prep_wo(wo_v, wof_s, wop_s, zvec):
    _store_tiles(wof_s, 0, wo_v[...].astype(f32))
    pieces = [_gather_rows(wof_s, d, D).astype(bf16) for d in range(16)]
    pieces.append(jnp.zeros((64, D), bf16))
    pieces += [_gather_rows(wof_s, d, D).astype(bf16) for d in (16, 17)]
    wopt = jnp.concatenate(pieces, axis=0).T
    wop_s[...] = _pk(wopt)
    return (pltpu.bitcast(wopt[D - 16:, 512:], i32) | pltpu.bitcast(wopt[D - 16:, :128], i32)) & zvec


def _kernel(xt_hbm, wqkv_hbm, wo_hbm, w1_hbm, b1_hbm, w2t_hbm, out_hbm,
            x_v, wqkv_v, wo_v, w1_v, b1_v, w2_v, xn_s, acc_s, a_s, wt_s, wp_s, wof_s, wop_s,
            qkv_s, o_s, out_v, s1_s, s2_s, sq_s, wr_s, l2_s, z_s, sem_in, sem_out):
    def cols(start, size):
        return pl.ds(_mo(start, 128), size)

    def tile(t):
        return cols(t * T, T)

    def prows(start, size):
        return pl.ds(_mo(start // 2, 64), size // 2)

    def xn_at(start, size):
        return _un(xn_s[prows(start, size), :])

    def cx(t):
        return pltpu.make_async_copy(xt_hbm.at[:, tile(t)], x_v.at[:, tile(t)], sem_in.at[8 + t])

    def cw(src, dst, lo, hi, k):
        return pltpu.make_async_copy(src.at[:, pl.ds(lo, hi - lo)], dst.at[:, pl.ds(lo, hi - lo)], sem_in.at[k])

    def out_copies(t, n):
        cs = cols(t * T + 128 * n, 128)
        if n < NB - 1:
            return [(0, D, pltpu.make_async_copy(out_v.at[:, cs], out_hbm.at[:, cs], sem_out.at[t * NOD + n]))]
        res, r0 = [], 0
        for k, r1 in enumerate(OSPLIT):
            res.append((r0, r1, pltpu.make_async_copy(out_v.at[r0:r1, cs], out_hbm.at[r0:r1, cs],
                                                      sem_out.at[t * NOD + n + k])))
            r0 = r1
        return res

    cb = pltpu.make_async_copy(b1_hbm, b1_v, sem_in.at[0])
    c1a = cw(w1_hbm, w1_v, 0, FH, 1)
    c1b = cw(w1_hbm, w1_v, FH, F1, 2)
    c2a = cw(w2t_hbm, w2_v, 0, F0, 3)
    cq = pltpu.make_async_copy(wqkv_hbm, wqkv_v, sem_in.at[4])
    co = pltpu.make_async_copy(wo_hbm, wo_v, sem_in.at[5])
    c1r = cw(w1_hbm, w1_v, F1, F, 6)
    c2r = cw(w2t_hbm, w2_v, F0, F, 7)
    for c in [cx(0), c1a, cb, c1b, c2a] + [cx(t) for t in range(1, NTILE)] + [cq, co, c1r, c2r]:
        c.start()

    z_s[0] = 0
    for i in range(4, 13):
        qkv_s[i, pl.ds(T, HALO), :] = jnp.zeros((HALO, 128), f32)
    qkv_s[13] = jnp.zeros((HALO + T, 128), f32)
    for part in range(3):
        wt_s[part, 4] = jnp.zeros(wt_s.shape[2:], f32)
    wof_s[4] = jnp.zeros(wof_s.shape[1:], f32)

    def zeros_vec():
        return jnp.full((8, 128), z_s[0], i32)

    def layernorm(start, ntok, blk):
        z = None
        res = []
        for b in range(ntok // blk):
            xt = _gate_f(x_v[:, cols(start + blk * b, blk)].astype(f32), z)
            xc = xt - jnp.mean(xt, axis=0, keepdims=True)
            v = jnp.mean(xc * xc, axis=0, keepdims=True)
            xn = (xc * jax.lax.rsqrt(v + EPS)).astype(bf16).T
            xn_s[prows(start + blk * b, blk), :] = _pk(xn)
            z = (pltpu.bitcast(xn[blk - 16:, 384:512], i32) | pltpu.bitcast(xn[blk - 16:, :128], i32)) & zeros_vec()
            res.append(xn)
        return jnp.concatenate(res, axis=0)

    def bias(c0):
        return b1_v[pl.ds(c0 // 128, 1), :].astype(f32)

    def ffn1(xnb, lo, hi, msplit):
        xa, xr = xnb[:, :512], xnb[:, 512:]
        mb = xnb.shape[0] // msplit
        rem = jnp.concatenate([_dot(xr[i * mb:(i + 1) * mb], w1_v[512:, lo:hi]) for i in range(msplit)], axis=0)
        outs = []
        for c0 in range(lo, hi, 128):
            h = _dot(xa, w1_v[:512, c0:c0 + 128])
            outs.append(_mish(h + (rem[:, c0 - lo:c0 - lo + 128] + bias(c0))))
        return _pk(jnp.concatenate(outs, axis=1).astype(bf16))

    def ffn2(a, lo, hi):
        return _dott(w2_v[:, lo:hi], _un(a))

    cx(0).wait()
    layernorm(0, HT, HT)
    c1a.wait()
    cb.wait()
    xnb0 = layernorm(HT, HT, HT)
    a_s[:HT // 2, :FH] = ffn1(xn_at(0, HT), 0, FH, 2)
    a_s[HT // 2:HT, :FH] = ffn1(xnb0, 0, FH, 2)
    c1b.wait()
    row8 = jax.lax.broadcasted_iota(i32, (8, 128), 0)
    for i in range(2 * NG):
        bv = jnp.broadcast_to(bias(F1 + 128 * i), (8, 128))
        wr_s[32:, 128 * i:128 * (i + 1)] = _zip_rows(jnp.where(row8 == 0, bv, 0.0), jnp.zeros((8, 128), f32))
    a_s[:HT, FH:] = ffn1(xn_at(0, T), FH, F1, 2)

    def p1_body(t, carry):
        @pl.when(t == 0)
        def _():
            c2a.wait()
        cx(t + 1).wait()
        xn = layernorm((t + 1) * T, T, 128)
        acc_s[:, tile(t)] = x_v[:, tile(t)].astype(f32) + ffn2(a_s[prows(t * T, T), :FA], 0, FA)
        for b in range(NB):
            a_s[prows((t + 1) * T + 128 * b, 128), :] = ffn1(xn[128 * b:128 * (b + 1)], 0, F1, 1)
        return carry

    jax.lax.fori_loop(0, NTILE - 1, p1_body, 0)

    cq.wait()
    co.wait()
    zv = zeros_vec()
    z = _prep_wo(wo_v, wof_s, wop_s, zv)
    for part in range(3):
        z = _prep_qkv(part, wqkv_v, wt_s.at[part], wp_s, zv, z)
    tl = NTILE - 1
    acc_s[:, tile(tl)] = x_v[:, tile(tl)].astype(f32) + ffn2(a_s[prows(tl * T, T), :F0], 0, F0)
    for t in range(NTILE - 1):
        acc_s[:, tile(t)] = acc_s[:, tile(t)] + ffn2(a_s[prows(t * T, T), FA:F0], FA, F0)
    c1r.wait()
    c2r.wait()

    def px_body(it, carry):
        def part(ref, base, n, al, axis=0):
            return ref.at[(slice(None),) * axis + (pl.ds(pl.multiple_of(base + it * n, al), n),)]

        z = [None]

        def piece(wds, sums_fn, dst):
            if z[0] is not None:
                zf = jnp.tile(z[0], (1, 2))
                wds[0], wds[3] = wds[0] | zf, wds[3] | zf
            blk = [_even_odd(_un(w)) for w in wds]
            sums = [sums_fn(*[b[par] for b in blk]) for par in range(2)]
            for n in range(5):
                v = _zip_rows(sums[0][n], sums[1][n])
                dst(n, v)
            z[0] = pltpu.bitcast(jnp.exp2(pltpu.bitcast(v[:, 128:] & zv, f32)), i32) & zv

        for w_v, s_s, hr, sums_fn in ((w1_v, s1_s, 256, _sums_b), (w2_v, s2_s, HD, _sums_a)):
            nr = hr // NPX
            wt, wb, sv = part(w_v, 0, nr, 16), part(w_v, hr, nr, 16), part(s_s, 0, nr // 2, 8, axis=1)
            for g0 in range(0, FS, 256):
                for r0 in range(0, nr, 16):
                    def dst(n, v, r0=r0, g0=g0, sv=sv):
                        sv[n, r0 // 2:r0 // 2 + 8, g0:g0 + 256] = v
                    piece([_pk(w[r0:r0 + 16, c0:c0 + 256]) for w in (wt, wb) for c0 in (F1 + g0, F1 + FS + g0)],
                          sums_fn, dst)
        nr = 384 // NPX
        wl, wr, sv = part(wp_s, 0, nr, 8), part(wp_s, 384, nr, 8), part(sq_s, 0, nr, 8, axis=1)
        for r0 in range(0, nr, 8):
            def dst(n, v, r0=r0):
                sv[n, r0:r0 + 8, :] = v
            piece([w[r0:r0 + 8, c0:c0 + 256] for c0 in (0, 256) for w in (wl, wr)], _sums_b, dst)

        l1 = {2: ((0, 0, 1),), 3: ((1, 1, 1),), 5: ((1, 0, 1), (0, 0, -1)), 6: ((0, 1, 1), (1, 1, -1))}
        q = FS // 2
        wq4 = [w2_v.at[pl.ds(pl.multiple_of(144 * k + 64 * it, 16), 80)] for k in range(4)]
        lv = l2_s.at[:, :, pl.ds(pl.multiple_of(32 * it, 8), 40)]
        for pi, n in enumerate(L2_PRE):
            for j in range(0, q, 128):
                for r0 in range(0, 80, 16):
                    blocks = []
                    for rq in range(2):
                        for cq_ in range(2):
                            blk = None
                            for rh, ch, sg in l1[n]:
                                c0 = F1 + ch * FS + cq_ * q + j
                                w = _pk(wq4[2 * rh + rq][r0:r0 + 16, c0:c0 + 128])
                                if blk is None and rq == cq_:
                                    w = w | z[0]
                                e = _even_odd(_un(w))
                                blk = e if blk is None else tuple(a + b if sg > 0 else a - b for a, b in zip(blk, e))
                            blocks.append(blk)
                    outs = [_sums_a(*[b[par] for b in blocks]) for par in range(2)]
                    for k in range(5):
                        v = _zip_rows(outs[0][k], outs[1][k])
                        lv[pi, k, r0 // 2:r0 // 2 + 8, j:j + 128] = v
                    z[0] = v & zv
        wr_s[:32, cols(it * FS, FS)] = _pk(w1_v[512:, cols(F1 + it * FS, FS)])
        nt = NTILE // NPX
        av, cv = part(a_s, 0, nt * HT, 64), part(acc_s, 0, nt * T, 128, axis=1)
        for t in range(nt):
            cv[:, t * T:(t + 1) * T] = cv[:, t * T:(t + 1) * T] + ffn2(av[t * HT:(t + 1) * HT, F0:], F0, F1)
        return carry

    jax.lax.fori_loop(0, NPX, px_body, 0)

    cexp_bits = pltpu.bitcast(jnp.full((8, 128), CEXP, f32), i32)

    def p2_body(t, carry):
        zvec = zeros_vec()
        xnb = xn_at(t * T, T)
        xe, xo = _even_odd(xnb)
        xf = jnp.concatenate([xe[:HT // 2], xo[:HT // 2], xe[HT // 2:], xo[HT // 2:]], axis=0)
        fb = xf[:HT, :256], xf[:HT, 256:512], xf[HT:, :256], xf[HT:, 256:512]
        x11, x22 = fb[0].astype(bf16), fb[3].astype(bf16)
        one = (jax.lax.broadcasted_iota(i32, (T, 16), 1) == 0).astype(f32)
        xr = jnp.concatenate([xf[:, 512:], one], axis=1).astype(bf16)
        xs = [v.astype(bf16) for v in _sums_a(*fb)]

        def h_products(g):
            lc, rc = 128 * g, FS + 128 * g
            sw = lambda n: _un(s1_s[n, :, lc:lc + 128])
            m1 = _dot(xs[0], sw(0))
            m2 = _dot(xs[1], w1_v[:256, F1 + lc:F1 + lc + 128])
            m3 = _dot(x11, sw(1))
            m4 = _dot(x22, sw(2))
            m5 = _dot(xs[2], w1_v[256:512, F1 + rc:F1 + rc + 128])
            m6 = _dot(xs[3], sw(3))
            m7 = _dot(xs[4], sw(4))
            rl = _dot(xr, _un(wr_s[:, lc:lc + 128]))
            rr = _dot(xr, _un(wr_s[:, rc:rc + 128]))
            return rl[:HT], rl[HT:], rr[:HT], rr[HT:], m1, m2, m3, m4, m5, m6, m7

        ptok = [None, None]

        def h_post(ms):
            outs = []
            for r0 in range(0, HT // 2, 8):
                ch = (r0 // 8) % 2
                o = []
                for rr0 in (r0, HT // 2 + r0):
                    rlt, rlb, rrt, rrb, m1, m2, m3, m4, m5, m6, m7 = [v[rr0:rr0 + 8] for v in ms]
                    m3, m4 = _gate_f(m3, ptok[ch]), _gate_f(m4, ptok[ch])
                    a12 = _mish((m3 + m5) + rrt)
                    a21 = _mish((m2 + m4) + rlb)
                    a11 = _mish((m1 + m4) + (m7 - m5) + rlt)
                    a22 = _mish((m1 - m2) + (m3 + m6) + rrb)
                    o.append((a11 + a22, a11, a21 - a22, a12 - a11, a22, a11 + a21, a12 + a22))
                    if rr0 == r0:
                        ptok[ch] = pltpu.bitcast(o[0][5] + o[0][6], i32) & zvec
                w = [_zip_rows(o[0][n], o[1][n]) for n in range(7)]
                outs.append(w)
                ptok[ch] = functools.reduce(lambda a, b: a | b, w) & zvec
            return [jnp.concatenate([o[n] for o in outs], axis=0) for n in range(7)]

        done = []
        prev = None
        for g in range(NG):
            cur = h_products(g)
            if prev is not None:
                done.append(h_post(prev))
            prev = cur

        for i in range(4, 14):
            qkv_s[i, pl.ds(0, HALO), :] = qkv_s[i, pl.ds(T, HALO), :]
        rem = _dott(_un(wp_s[pl.ds(768, 96), :]), xnb).T
        qkv_s[12, pl.ds(HALO, T), :] = rem[:, :128]
        qkv_s[13, pl.ds(HALO, T), :64] = rem[:, 128:]
        n11, n12, n21, n22 = xnb[:HT, :256], xnb[:HT, 256:512], xnb[HT:, :256], xnb[HT:, 256:512]
        ns = [(p.astype(f32) + sg * q.astype(f32)).astype(bf16) for p, q, sg in
              ((n11, n22, 1.0), (n21, n22, 1.0), (n11, n12, 1.0), (n21, n11, -1.0), (n12, n22, -1.0))]
        nrem = xnb[:, 512:]
        for i in range(6):
            wl = lambda lo, hi: _un(wp_s[pl.ds(64 * i, 64), lo:hi])
            wr = lambda lo, hi: _un(wp_s[pl.ds(384 + 64 * i, 64), lo:hi])
            sw = lambda n: _un(sq_s[n, pl.ds(64 * i, 64), :])
            rl, rr = _dott(nrem, wl(512, D)), _dott(nrem, wr(512, D))
            m3, m5 = _dott(n11, sw(1)), _dott(ns[2], wr(256, 512))
            m4, m2 = _dott(n22, sw(2)), _dott(ns[1], wl(0, 256))
            m1, m7, m6 = _dott(ns[0], sw(0)), _dott(ns[4], sw(4)), _dott(ns[3], sw(3))
            qkv_s[6 + i, pl.ds(HALO, HT), :] = (m3 + m5) + rr[:HT]
            qkv_s[i, pl.ds(HALO + HT, HT), :] = (m2 + m4) + rl[HT:]
            qkv_s[i, pl.ds(HALO, HT), :] = (m1 + m4) + (m7 - m5) + rl[:HT]
            qkv_s[6 + i, pl.ds(HALO + HT, HT), :] = (m1 - m2) + (m3 + m6) + rr[HT:]
        done.append(h_post(prev))

        def ld(i, r):
            return qkv_s[i, pl.ds(r, 8), :]

        def token(x):
            return pltpu.bitcast(x, i32) & zvec

        def qk(j, z):
            r = HALO + 8 * j
            scale = pltpu.bitcast(cexp_bits if z is None else cexp_bits | z, f32)
            q = [ld(i, r) * scale for i in (0, 1, 2, 3, 12)]
            raw = []
            for w in range(W):
                k = [ld(i, r - DIL * w) for i in (4, 5, 6, 7, 13)]
                raw.append((q[0] * k[0] + q[1] * k[1]) + (q[2] * k[2] + q[3] * k[3]) + q[4] * k[4])
            return raw

        def softmax(j, raw):
            s = []
            for w, sw in enumerate(raw):
                sw = (sw + pltpu.roll(sw, 64, 1)) + (pltpu.roll(sw, 32, 1) + pltpu.roll(sw, 96, 1))
                if 8 * j < DIL * w:
                    sw = jnp.where(row8 + (t * T + 8 * j - DIL * w) >= 0, sw, NEG)
                s.append(sw)
            mx = functools.reduce(jnp.maximum, s)
            e = [jnp.exp2(sw - mx) for sw in s]
            return e, pl.reciprocal(functools.reduce(lambda a, b: a + b, e), approx=True)

        def pv(j, e, rinv, z):
            r = HALO + 8 * j
            for oi, i in enumerate((8, 9, 10, 11, 12)):
                p = _gate_f(e[0], z) * ld(i, r)
                for w in range(1, W):
                    p = p + e[w] * ld(i, r - DIL * w)
                o = p * rinv
                o_s[pl.ds(8 * j, 8), pl.ds(128 * oi, 128)] = o
                z = token(o)

        raws = {0: qk(0, None)}
        raws[1] = qk(1, token(raws[0][W - 1]))
        for j in range(T // 8):
            e, rinv = softmax(j, raws.pop(j))
            zq = None
            if j + 2 < T // 8:
                raws[j + 2] = qk(j + 2, token(rinv))
                zq = token(raws[j + 2][W - 1])
            pv(j, e, rinv, zq)

        hg, q = NG // 2, FS // 2
        lhs = (s2_s[0], s2_s[1], _pk(w2_v[:HD, F1:F1 + FS]), _pk(w2_v[HD:, F1 + FS:]), s2_s[2], s2_s[3], s2_s[4])
        z = ptok[0] | ptok[1]
        rhs2 = {}
        for n in L2_ORDER:
            cols_ = [[] for _ in range(5)]
            for g in range(hg):
                rows_ = [[] for _ in range(5)]
                for r in range(0, 64, 8):
                    w11, w12 = done[g][n][r:r + 8], done[g][n][64 + r:72 + r]
                    w21, w22 = done[g + hg][n][r:r + 8], done[g + hg][n][64 + r:72 + r]
                    u11, u12, u21, u22 = [_even_odd(_un(w)) for w in (w11 | z, w12, w21, w22 | z)]
                    o = [_zip_rows(u11[0] + u22[0], u11[1] + u22[1]), _zip_rows(u12[0] - u22[0], u12[1] - u22[1]),
                         _zip_rows(u21[0] - u11[0], u21[1] - u11[1]), _zip_rows(u11[0] + u12[0], u11[1] + u12[1]),
                         _zip_rows(u21[0] + u22[0], u21[1] + u22[1])]
                    for k in range(5):
                        rows_[k].append(o[k])
                    z = functools.reduce(lambda a, b: a | b, o) & zvec
                for k in range(5):
                    cols_[k].append(jnp.concatenate(rows_[k], axis=0))
            sm = [jnp.concatenate(cc, axis=1) for cc in cols_]
            b11 = jnp.concatenate([done[g][n][:64] for g in range(hg)], axis=1)
            b22 = jnp.concatenate([done[g + hg][n][64:] for g in range(hg)], axis=1)
            rhs2[n] = (sm[0], b11, sm[1], sm[2], b22, sm[3], sm[4])

        def wsum(a, b, sg):
            (ae, ao), (be, bo) = _even_odd(_un(a)), _even_odd(_un(b))
            return _zip_rows(ae + be, ao + bo) if sg > 0 else _zip_rows(ae - be, ao - bo)

        ms = [None] * 7
        for n in L2_ORDER:
            a11, a12, a21, a22 = lhs[n][:72, :q], lhs[n][:72, q:], lhs[n][72:, :q], lhs[n][72:, q:]
            if n in L2_PRE:
                lp = lambda k: l2_s[L2_PRE.index(n), k]
                l2 = (lp(0), lp(1), a11, a22, lp(2), lp(3), lp(4))
            else:
                l2 = (wsum(a11, a22, 1), wsum(a21, a22, 1), a11, a22,
                      wsum(a11, a12, 1), wsum(a21, a11, -1), wsum(a12, a22, -1))
            ms[n] = _combine(*[_dott(_un(l2[k]), _un(rhs2[n][k])) for k in range(7)])
        acc = acc_s[:, tile(t)] + _combine(*ms)

        ob = o_s[...].astype(bf16)
        wop = _un(wop_s[...])
        for n in range(NB):
            cs = cols(t * T + 128 * n, 128)
            fin = (acc[:, 128 * n:128 * (n + 1)] + _dott(wop, ob[128 * n:128 * (n + 1)])).astype(bf16)
            for r0, r1, cp in out_copies(t, n):
                out_v[r0:r1, cs] = fin[r0:r1]
                cp.start()
        return carry

    jax.lax.fori_loop(0, NTILE, p2_body, 0)
    for t in range(NTILE):
        for n in range(NB):
            for _, _, cp in out_copies(t, n):
                cp.wait()


@jax.jit
def pallas_parallel_sum__sliding_local_dilated__dense_activation_mish__prompt_kernel(
    A_x: jax.Array,
    A_wqkv: jax.Array,
    A_wo: jax.Array,
    B_x: jax.Array,
    B_w1: jax.Array,
    B_b1: jax.Array,
    B_w2: jax.Array,
):
    del B_x
    hbm = pl.BlockSpec(memory_space=pl.ANY)
    out_t = pl.pallas_call(
        _kernel,
        in_specs=[hbm] * 6,
        out_specs=hbm,
        out_shape=jax.ShapeDtypeStruct((D, S), bf16),
        scratch_shapes=[
            pltpu.VMEM((D, S), bf16),
            pltpu.VMEM((D, 3 * D), bf16),
            pltpu.VMEM((D, D), bf16),
            pltpu.VMEM((D, F), bf16),
            pltpu.VMEM((F // 128, 128), bf16),
            pltpu.VMEM((D, F), bf16),
            pltpu.VMEM((S // 2, D), i32),
            pltpu.VMEM((D, S), f32),
            pltpu.VMEM((S // 2, F1), i32),
            pltpu.VMEM((3, 5, 640, 128), f32),
            pltpu.VMEM((3 * D // 2, D), i32),
            pltpu.VMEM((5, D, 128), f32),
            pltpu.VMEM((D // 2, 640), i32),
            pltpu.VMEM((14, HALO + T, 128), f32),
            pltpu.VMEM((T, 640), f32),
            pltpu.VMEM((D, S), bf16),
            pltpu.VMEM((5, 128, FS), i32),
            pltpu.VMEM((5, HD // 2, FS), i32),
            pltpu.VMEM((5, 384, 256), i32),
            pltpu.VMEM((40, 2 * FS), i32),
            pltpu.VMEM((len(L2_PRE), 5, 72, FS // 2), i32),
            pltpu.SMEM((1,), i32),
            pltpu.SemaphoreType.DMA((8 + NTILE,)),
            pltpu.SemaphoreType.DMA((NTILE * NOD,)),
        ],
        compiler_params=pltpu.CompilerParams(vmem_limit_bytes=100 * 1024 * 1024),
    )(A_x.reshape(S, D).T, A_wqkv, A_wo, B_w1, B_b1.reshape(F // 128, 128), B_w2.T)
    return out_t.T.reshape(1, S, D)
```

```python
import functools

import jax
import jax.numpy as jnp
import jax.experimental.pallas as pl
import jax.experimental.pallas.tpu as pltpu

S, D, F = 2048, 576, 4608
H, DH, W, DIL = 32, 18, 8, 2
T = 512
HT, HD = T // 2, D // 2
NTILE = S // T
NB = T // 128
HALO = 16
FH = 256
FA = 128
F0 = 384
F1 = 1024
FS = (F - F1) // 2
NG = FS // 128
NPX = 2
L2_ORDER = (2, 3, 6, 5, 0, 1, 4)
L2_PRE = (2, 3, 6, 5)
KPAIRS = ((0, 2, 2), (4, 6, 2), (8, 10, 2), (12, 13, 1))
KT = tuple(tuple(kp[h] + c for kp in KPAIRS for c in range(kp[2])) for h in range(2))
OSPLIT = (384, D)
NOD = NB - 1 + len(OSPLIT)
EPS = 1e-5
LOG2E = 1.4426950408889634
CEXP = DH ** -0.5 * LOG2E
NEG = -1e9 * LOG2E
f32, bf16, i32 = jnp.float32, jnp.bfloat16, jnp.int32
NT = (((1,), (1,)), ((), ()))


def _mo(v, n):
    return v if isinstance(v, int) else pl.multiple_of(v, n)


def _pk(x):
    return pltpu.bitcast(x, i32)


def _un(x):
    return pltpu.bitcast(x, bf16)


def _opnd(ref, idx, tiles, rows=None):
    w = ref.bitcast(i32)
    rs = slice(None) if rows is None else slice(rows[0] // 2, rows[1] // 2)
    return jnp.concatenate([_un(w[idx + (t, rs)]) for t in tiles], axis=1)


def _dot(a, b):
    return jnp.dot(a, b, preferred_element_type=f32)


def _dott(a, b):
    return jax.lax.dot_general(a, b, NT, preferred_element_type=f32)


def _sums_a(p11, p12, p21, p22):
    return p11 + p22, p21 + p22, p11 + p12, p21 - p11, p12 - p22


def _sums_b(p11, p12, p21, p22):
    return p11 + p22, p12 - p22, p21 - p11, p11 + p12, p21 + p22


def _combine(m1, m2, m3, m4, m5, m6, m7):
    return jnp.concatenate(
        [jnp.concatenate([(m1 + m4) + (m7 - m5), m3 + m5], axis=1),
         jnp.concatenate([m2 + m4, (m1 - m2) + (m3 + m6)], axis=1)], axis=0)


def _mish(h):
    u = jnp.exp(jnp.minimum(h, 20.0))
    n = u * (u + 2.0)
    return h * (n * pl.reciprocal(n + 2.0, approx=True))


def _gate(x, z, rows, dtype):
    if z is None:
        return x
    head = pltpu.bitcast(pltpu.bitcast(x[:rows, :128], i32) | z, dtype)
    if x.shape[1] > 128:
        head = jnp.concatenate([head, x[:rows, 128:]], axis=1)
    return jnp.concatenate([head, x[rows:]], axis=0) if x.shape[0] > rows else head


def _gate_f(x, z):
    return _gate(x, z, 8, f32)


def _gate_all(x, z):
    if z is None:
        return x
    return pltpu.bitcast(pltpu.bitcast(x, i32) | jnp.tile(z, (x.shape[0] // 8, x.shape[1] // 128)), f32)


def _gate_b(x, z):
    return _gate(x, z, 16, bf16)


def _wp_row(part, d):
    if d < 16:
        return part * 512 + d * 32
    return {0: 1536, 2: 1600, 1: 1664}[part] + (d - 16) * 32


def _gather_rows(s, start, width):
    parts = []
    for i in range(s.shape[0]):
        parts.append(s[i, pl.ds(start, H, stride=DH), :][:, :min(128, width - 128 * i)])
    return jnp.concatenate(parts, axis=1)


def _store_tiles(s, r0, val):
    for i in range(s.shape[0]):
        w = min(128, val.shape[1] - 128 * i)
        s[i, pl.ds(r0, val.shape[0]), :w] = val[:, 128 * i:128 * i + w]


def _prep_qkv(part, wqkv_v, wt_s, wp_s, zvec, z):
    lo = (part * D) // 128 * 128
    hi = min(-(-((part + 1) * D) // 128) * 128, 3 * D)
    for c0 in range(lo, hi, 128):
        cw = min(128, hi - c0)
        blk = wqkv_v[:, c0:c0 + cw]
        if cw == 128:
            blk = _gate_b(blk, z)
        wt = blk.T.astype(f32)
        _store_tiles(wt_s, c0 - lo, wt)
        z = pltpu.bitcast(wt[cw - 8:, 384:512], i32) & zvec
    for d in range(DH):
        rows = _gather_rows(wt_s, part * D - lo + d, D)
        if d % 3 == 0:
            rows = _gate_f(rows, z)
        rows = rows.astype(bf16)
        _store_tiles(wp_s, _wp_row(part, d), rows)
        z = pltpu.bitcast(rows[:16, :128], i32) & zvec
    return z


def _prep_wo(wo_v, wof_s, wop_s, zvec):
    _store_tiles(wof_s, 0, wo_v[...].astype(f32))
    pieces = [_gather_rows(wof_s, d, D).astype(bf16) for d in range(16)]
    pieces.append(jnp.zeros((64, D), bf16))
    pieces += [_gather_rows(wof_s, d, D).astype(bf16) for d in (16, 17)]
    wopt = jnp.concatenate(pieces, axis=0).T
    wop_s[...] = _pk(wopt)
    return (pltpu.bitcast(wopt[D - 16:, 512:], i32) | pltpu.bitcast(wopt[D - 16:, :128], i32)) & zvec


def _kernel(xt_hbm, wqkv_hbm, wo_hbm, w1_hbm, b1_hbm, w2t_hbm, out_hbm,
            x_v, wqkv_v, wo_v, w1_v, b1_v, w2_v, xn_s, acc_s, a_s, wt_s, wp_s, wof_s, wop_s,
            qkv_s, o_s, out_v, s1_s, s2_s, sq_s, wr_s, l2_s, op_s, r2_s, z_s, sem_in, sem_out):
    def cols(start, size):
        return pl.ds(_mo(start, 128), size)

    def tile(t):
        return cols(t * T, T)

    def prows(start, size):
        return pl.ds(_mo(start // 2, 64), size // 2)

    def xn_at(start, size):
        return _un(xn_s[prows(start, size), :])

    def cx(t):
        return pltpu.make_async_copy(xt_hbm.at[:, tile(t)], x_v.at[:, tile(t)], sem_in.at[8 + t])

    def cw(src, dst, lo, hi, k):
        return pltpu.make_async_copy(src.at[:, pl.ds(lo, hi - lo)], dst.at[:, pl.ds(lo, hi - lo)], sem_in.at[k])

    def out_copies(t, n):
        cs = cols(t * T + 128 * n, 128)
        if n < NB - 1:
            return [(0, D, pltpu.make_async_copy(out_v.at[:, cs], out_hbm.at[:, cs], sem_out.at[t * NOD + n]))]
        res, r0 = [], 0
        for k, r1 in enumerate(OSPLIT):
            res.append((r0, r1, pltpu.make_async_copy(out_v.at[r0:r1, cs], out_hbm.at[r0:r1, cs],
                                                      sem_out.at[t * NOD + n + k])))
            r0 = r1
        return res

    cb = pltpu.make_async_copy(b1_hbm, b1_v, sem_in.at[0])
    c1a = cw(w1_hbm, w1_v, 0, FH, 1)
    c1b = cw(w1_hbm, w1_v, FH, F1, 2)
    c2a = cw(w2t_hbm, w2_v, 0, F0, 3)
    cq = pltpu.make_async_copy(wqkv_hbm, wqkv_v, sem_in.at[4])
    co = pltpu.make_async_copy(wo_hbm, wo_v, sem_in.at[5])
    c1r = cw(w1_hbm, w1_v, F1, F, 6)
    c2r = cw(w2t_hbm, w2_v, F0, F, 7)
    for c in [cx(0), c1a, cb, c1b, c2a] + [cx(t) for t in range(1, NTILE)] + [cq, co, c1r, c2r]:
        c.start()

    z_s[0] = 0
    for i in range(4, 13):
        qkv_s[i, pl.ds(T, HALO), :] = jnp.zeros((HALO, 128), f32)
    qkv_s[13] = jnp.zeros((HALO + T, 128), f32)
    for part in range(3):
        wt_s[part, 4] = jnp.zeros(wt_s.shape[2:], f32)
    wof_s[4] = jnp.zeros(wof_s.shape[1:], f32)
    wp_s[4] = jnp.zeros(wp_s.shape[1:], bf16)

    def zeros_vec():
        return jnp.full((8, 128), z_s[0], i32)

    def layernorm(start, ntok, blk):
        z = None
        res = []
        for b in range(ntok // blk):
            xt = _gate_f(x_v[:, cols(start + blk * b, blk)].astype(f32), z)
            xc = xt - jnp.mean(xt, axis=0, keepdims=True)
            v = jnp.mean(xc * xc, axis=0, keepdims=True)
            xn = (xc * jax.lax.rsqrt(v + EPS)).astype(bf16).T
            xn_s[prows(start + blk * b, blk), :] = _pk(xn)
            z = (pltpu.bitcast(xn[blk - 16:, 384:512], i32) | pltpu.bitcast(xn[blk - 16:, :128], i32)) & zeros_vec()
            res.append(xn)
        return jnp.concatenate(res, axis=0)

    def bias(c0):
        return b1_v[pl.ds(c0 // 128, 1), :].astype(f32)

    def ffn1(xnb, lo, hi, msplit):
        xa, xr = xnb[:, :512], xnb[:, 512:]
        mb = xnb.shape[0] // msplit
        rem = jnp.concatenate([_dot(xr[i * mb:(i + 1) * mb], w1_v[512:, lo:hi]) for i in range(msplit)], axis=0)
        outs = []
        for c0 in range(lo, hi, 128):
            h = _dot(xa, w1_v[:512, c0:c0 + 128])
            outs.append(_mish(h + (rem[:, c0 - lo:c0 - lo + 128] + bias(c0))))
        return _pk(jnp.concatenate(outs, axis=1).astype(bf16))

    def ffn2(a, lo, hi):
        return _dott(w2_v[:, lo:hi], _un(a))

    cx(0).wait()
    layernorm(0, HT, HT)
    c1a.wait()
    cb.wait()
    xnb0 = layernorm(HT, HT, HT)
    a_s[:HT // 2, :FH] = ffn1(xn_at(0, HT), 0, FH, 2)
    a_s[HT // 2:HT, :FH] = ffn1(xnb0, 0, FH, 2)
    c1b.wait()
    row8 = jax.lax.broadcasted_iota(i32, (8, 128), 0)
    first = jax.lax.broadcasted_iota(i32, (16, 128), 0) == 0
    for i in range(2 * NG):
        wr_s[i, 64:] = jnp.where(first, jnp.broadcast_to(bias(F1 + 128 * i), (16, 128)), 0.0).astype(bf16)
    a_s[:HT, FH:] = ffn1(xn_at(0, T), FH, F1, 2)

    def p1_body(t, carry):
        @pl.when(t == 0)
        def _():
            c2a.wait()
        cx(t + 1).wait()
        xn = layernorm((t + 1) * T, T, 128)
        acc_s[:, tile(t)] = x_v[:, tile(t)].astype(f32) + ffn2(a_s[prows(t * T, T), :FA], 0, FA)
        for b in range(NB):
            a_s[prows((t + 1) * T + 128 * b, 128), :] = ffn1(xn[128 * b:128 * (b + 1)], 0, F1, 1)
        return carry

    jax.lax.fori_loop(0, NTILE - 1, p1_body, 0)

    cq.wait()
    co.wait()
    zv = zeros_vec()
    z = _prep_wo(wo_v, wof_s, wop_s, zv)
    for part in range(3):
        z = _prep_qkv(part, wqkv_v, wt_s.at[part], wp_s, zv, z)
    tl = NTILE - 1
    acc_s[:, tile(tl)] = x_v[:, tile(tl)].astype(f32) + ffn2(a_s[prows(tl * T, T), :F0], 0, F0)
    for t in range(NTILE - 1):
        acc_s[:, tile(t)] = acc_s[:, tile(t)] + ffn2(a_s[prows(t * T, T), FA:F0], FA, F0)
    c1r.wait()
    c2r.wait()

    def px_body(it, carry):
        def part(ref, base, n, al, axis=0):
            return ref.at[(slice(None),) * axis + (pl.ds(pl.multiple_of(base + it * n, al), n),)]

        z = [None]

        def piece(blk, sums_fn, dst, hop):
            blk[0], blk[3] = _gate_all(blk[0], z[0]), _gate_all(blk[3], z[0])
            sums = sums_fn(*blk)
            for n in range(5):
                for c in range(sums[n].shape[1] // 128):
                    dst(n, c, sums[n][:, 128 * c:128 * (c + 1)].astype(bf16))
            z[0] = pltpu.bitcast(sums[4][8:, :128] + sums[3][8:, :128], i32) & zv
            for _ in range(hop):
                z[0] = pltpu.bitcast(jnp.exp2(pltpu.bitcast(z[0], f32)), i32) & zv

        for w_v, s_s, hr, sums_fn in ((w1_v, s1_s, 256, _sums_b), (w2_v, s2_s, HD, _sums_a)):
            nr = hr // NPX
            wt, wb, sv = part(w_v, 0, nr, 16), part(w_v, hr, nr, 16), part(s_s, 0, nr, 16, axis=2)
            for g in range(0, NG, 2):
                for r0 in range(0, nr, 16):
                    def dst(n, c, v, r0=r0, g=g, sv=sv):
                        sv[n, g + c, r0:r0 + 16] = v
                    piece([w[r0:r0 + 16, c0:c0 + 256].astype(f32) for w in (wt, wb)
                           for c0 in (F1 + 128 * g, F1 + FS + 128 * g)], sums_fn, dst, 1)
        nr = 768 // NPX
        wl, wr, sv = part(wp_s, 0, nr, 16, axis=1), part(wp_s, 768, nr, 16, axis=1), part(sq_s, 0, nr, 16, axis=2)
        for r0 in range(0, nr, 16):
            def dst(n, c, v, r0=r0):
                sv[n, c, r0:r0 + 16] = v
            piece([jnp.concatenate([w[k, r0:r0 + 16].astype(f32) for k in (k0, k0 + 1)], axis=1)
                   for k0 in (0, 2) for w in (wl, wr)], _sums_b, dst, 1)

        l1 = {2: ((0, 0, 1),), 3: ((1, 1, 1),), 5: ((1, 0, 1), (0, 0, -1)), 6: ((0, 1, 1), (1, 1, -1))}
        wq4 = [w2_v.at[pl.ds(pl.multiple_of(144 * k + 64 * it, 16), 80)] for k in range(4)]
        lv = l2_s.at[:, :, :, pl.ds(pl.multiple_of(64 * it, 16), 80)]
        for pi, n in enumerate(L2_PRE):
            for j, (ka, kb, wd) in enumerate(KPAIRS):
                for r0 in range(0, 80, 16):
                    blocks = []
                    for rq in range(2):
                        for kc in (ka, kb):
                            blk = None
                            for rh, ch, sg in l1[n]:
                                c0 = F1 + ch * FS + 128 * kc
                                e = wq4[2 * rh + rq][r0:r0 + 16, c0:c0 + 128 * wd].astype(f32)
                                blk = e if blk is None else (blk + e if sg > 0 else blk - e)
                            blocks.append(blk)
                    def dst(k, c, v, r0=r0, j=j, pi=pi):
                        lv[pi, k, 2 * j + c, r0:r0 + 16] = v
                    piece(blocks, _sums_a, dst, 2)
        wv, rv = w1_v.at[512:, cols(F1 + it * FS, FS)], part(wr_s, 0, NG, 1)
        for g in range(NG):
            rv[g, :64] = wv[:, 128 * g:128 * (g + 1)]
        nt = NTILE // NPX
        av, cv = part(a_s, 0, nt * HT, 64), part(acc_s, 0, nt * T, 128, axis=1)
        for t in range(nt):
            cv[:, t * T:(t + 1) * T] = cv[:, t * T:(t + 1) * T] + ffn2(av[t * HT:(t + 1) * HT, F0:], F0, F1)
        return carry

    jax.lax.fori_loop(0, NPX, px_body, 0)

    cexp_bits = pltpu.bitcast(jnp.full((8, 128), CEXP, f32), i32)

    def p2_body(t, carry):
        zvec = zeros_vec()
        xnb = xn_at(t * T, T)
        x11, x12, x21, x22 = xnb[:HT, :256], xnb[:HT, 256:512], xnb[HT:, :256], xnb[HT:, 256:512]
        xs = [v.astype(bf16) for v in _sums_a(*[v.astype(f32) for v in (x11, x12, x21, x22)])]
        one = (jax.lax.broadcasted_iota(i32, (T, 16), 1) == 0).astype(f32)
        xr = jnp.concatenate([xnb[:, 512:].astype(f32), one], axis=1).astype(bf16)

        def h_products(g):
            lc, rc = 128 * g, FS + 128 * g
            sw = lambda n: _opnd(s1_s, (n,), (g,))
            m1 = _dot(xs[0], sw(0))
            m2 = _dot(xs[1], w1_v[:256, F1 + lc:F1 + lc + 128])
            m3 = _dot(x11, sw(1))
            m4 = _dot(x22, sw(2))
            m5 = _dot(xs[2], w1_v[256:512, F1 + rc:F1 + rc + 128])
            m6 = _dot(xs[3], sw(3))
            m7 = _dot(xs[4], sw(4))
            rl = _dot(xr, _opnd(wr_s, (), (g,)))
            rr = _dot(xr, _opnd(wr_s, (), (NG + g,)))
            return rl[:HT], rl[HT:], rr[:HT], rr[HT:], m1, m2, m3, m4, m5, m6, m7

        ptok = [None, None]
        op_w, r2_w = op_s.bitcast(i32), r2_s.bitcast(i32)

        def h_post(g, ms):
            for r0 in range(0, HT, 16):
                ch = (r0 // 16) % 2
                o = []
                for rr0 in (r0, r0 + 8):
                    rlt, rlb, rrt, rrb, m1, m2, m3, m4, m5, m6, m7 = [v[rr0:rr0 + 8] for v in ms]
                    m5, m2 = _gate_f(m5, ptok[ch]), _gate_f(m2, ptok[ch])
                    a12 = _mish((m3 + m5) + rrt)
                    a21 = _mish((m2 + m4) + rlb)
                    a11 = _mish((m1 + m4) + (m7 - m5) + rlt)
                    a22 = _mish((m1 - m2) + (m3 + m6) + rrb)
                    o.append((a11 + a22, a11, a21 - a22, a12 - a11, a22, a11 + a21, a12 + a22))
                    if rr0 == r0:
                        ptok[ch] = pltpu.bitcast(o[0][5] + o[0][6], i32) & zvec
                for n in range(7):
                    op_s[n, g, r0:r0 + 16] = jnp.concatenate([o[0][n], o[1][n]], axis=0).astype(bf16)
                w = [op_w[n, g, r0 // 2:r0 // 2 + 8] for n in range(7)]
                ptok[ch] = functools.reduce(lambda a, b: a | b, w) & zvec

        prev = None
        for g in range(NG):
            cur = (g, h_products(g))
            if prev is not None:
                h_post(*prev)
            prev = cur

        for i in range(4, 14):
            qkv_s[i, pl.ds(0, HALO), :] = qkv_s[i, pl.ds(T, HALO), :]
        rem = _dott(_opnd(wp_s, (), range(5), (1536, 1728))[:, :D], xnb).T
        qkv_s[12, pl.ds(HALO, T), :] = rem[:, :128]
        qkv_s[13, pl.ds(HALO, T), :64] = rem[:, 128:]
        nrem = xnb[:, 512:]
        for i in range(6):
            wl = lambda ks: _opnd(wp_s, (), ks, (128 * i, 128 * (i + 1)))
            wr = lambda ks: _opnd(wp_s, (), ks, (768 + 128 * i, 768 + 128 * (i + 1)))
            sw = lambda n: _opnd(sq_s, (n,), (0, 1), (128 * i, 128 * (i + 1)))
            rl, rr = _dott(nrem, wl((4,))[:, :64]), _dott(nrem, wr((4,))[:, :64])
            m3, m5 = _dott(x11, sw(1)), _dott(xs[2], wr((2, 3)))
            m4, m2 = _dott(x22, sw(2)), _dott(xs[1], wl((0, 1)))
            m1, m7, m6 = _dott(xs[0], sw(0)), _dott(xs[4], sw(4)), _dott(xs[3], sw(3))
            qkv_s[6 + i, pl.ds(HALO, HT), :] = (m3 + m5) + rr[:HT]
            qkv_s[i, pl.ds(HALO + HT, HT), :] = (m2 + m4) + rl[HT:]
            qkv_s[i, pl.ds(HALO, HT), :] = (m1 + m4) + (m7 - m5) + rl[:HT]
            qkv_s[6 + i, pl.ds(HALO + HT, HT), :] = (m1 - m2) + (m3 + m6) + rr[HT:]
        h_post(*prev)

        def ld(i, r):
            return qkv_s[i, pl.ds(r, 8), :]

        def token(x):
            return pltpu.bitcast(x, i32) & zvec

        def qk(j, z):
            r = HALO + 8 * j
            scale = pltpu.bitcast(cexp_bits if z is None else cexp_bits | z, f32)
            q = [ld(i, r) * scale for i in (0, 1, 2, 3, 12)]
            raw = []
            for w in range(W):
                k = [ld(i, r - DIL * w) for i in (4, 5, 6, 7, 13)]
                raw.append((q[0] * k[0] + q[1] * k[1]) + (q[2] * k[2] + q[3] * k[3]) + q[4] * k[4])
            return raw

        def softmax(j, raw):
            s = []
            for w, sw in enumerate(raw):
                sw = (sw + pltpu.roll(sw, 64, 1)) + (pltpu.roll(sw, 32, 1) + pltpu.roll(sw, 96, 1))
                if 8 * j < DIL * w:
                    sw = jnp.where(row8 + (t * T + 8 * j - DIL * w) >= 0, sw, NEG)
                s.append(sw)
            mx = functools.reduce(jnp.maximum, s)
            e = [jnp.exp2(sw - mx) for sw in s]
            return e, pl.reciprocal(functools.reduce(lambda a, b: a + b, e), approx=True)

        def pv(j, e, rinv, z):
            r = HALO + 8 * j
            for oi, i in enumerate((8, 9, 10, 11, 12)):
                p = _gate_f(e[0], z) * ld(i, r)
                for w in range(1, W):
                    p = p + e[w] * ld(i, r - DIL * w)
                o = p * rinv
                o_s[pl.ds(8 * j, 8), pl.ds(128 * oi, 128)] = o
                z = token(o)

        raws = {0: qk(0, None)}
        raws[1] = qk(1, token(raws[0][W - 1]))
        for j in range(T // 8):
            e, rinv = softmax(j, raws.pop(j))
            zq = None
            if j + 2 < T // 8:
                raws[j + 2] = qk(j + 2, token(rinv))
                zq = token(raws[j + 2][W - 1])
            pv(j, e, rinv, zq)

        z = ptok[0] | ptok[1]
        for n in L2_ORDER:
            for j in range(NG // 2):
                for r in range(0, 128, 16):
                    u = [op_w[n, kt[j], r1 // 2:r1 // 2 + 8] for kt in KT for r1 in (r, 128 + r)]
                    o = _sums_b(*[_un(w).astype(f32) for w in (u[0] | z, u[1], u[2], u[3] | z)])
                    for k in range(5):
                        r2_s[n, k, j, r:r + 16] = o[k].astype(bf16)
                    z = functools.reduce(lambda a, b: a | b, [r2_w[n, k, j, r // 2:r // 2 + 8] for k in range(5)]) & zvec

        def lhs1(n, rh, kh):
            r0 = 144 * rh
            if n in (2, 3):
                r0, c0 = r0 + (n - 2) * HD, F1 + (n - 2) * FS
                return jnp.concatenate([w2_v[r0:r0 + 144, c0 + 128 * k:c0 + 128 * (k + 1)] for k in KT[kh]], axis=1)
            return _opnd(s2_s, ({0: 0, 1: 1, 4: 2, 5: 3, 6: 4}[n],), KT[kh], (r0, r0 + 144))

        ms = [None] * 7
        for n in L2_ORDER:
            a11, a22 = lhs1(n, 0, 0), lhs1(n, 1, 1)
            if n in L2_PRE:
                sm = [_opnd(l2_s, (L2_PRE.index(n), k), range(NG // 2)) for k in range(5)]
            else:
                sm = [v.astype(bf16) for v in
                      _sums_a(*[v.astype(f32) for v in (a11, lhs1(n, 0, 1), lhs1(n, 1, 0), a22)])]
            l2 = (sm[0], sm[1], a11, a22, sm[2], sm[3], sm[4])
            rs = [_opnd(r2_s, (n, k), range(NG // 2)) for k in range(5)]
            r2 = (rs[0], _opnd(op_s, (n,), KT[0], (0, 128)), rs[1], rs[2], _opnd(op_s, (n,), KT[1], (128, HT)), rs[3], rs[4])
            ms[n] = _combine(*[_dott(l2[k], r2[k]) for k in range(7)])
        acc = acc_s[:, tile(t)] + _combine(*ms)

        ob = o_s[...].astype(bf16)
        wop = _un(wop_s[...])
        for n in range(NB):
            cs = cols(t * T + 128 * n, 128)
            fin = (acc[:, 128 * n:128 * (n + 1)] + _dott(wop, ob[128 * n:128 * (n + 1)])).astype(bf16)
            for r0, r1, cp in out_copies(t, n):
                out_v[r0:r1, cs] = fin[r0:r1]
                cp.start()
        return carry

    jax.lax.fori_loop(0, NTILE, p2_body, 0)
    for t in range(NTILE):
        for n in range(NB):
            for _, _, cp in out_copies(t, n):
                cp.wait()


@jax.jit
def pallas_parallel_sum__sliding_local_dilated__dense_activation_mish__prompt_kernel(
    A_x: jax.Array,
    A_wqkv: jax.Array,
    A_wo: jax.Array,
    B_x: jax.Array,
    B_w1: jax.Array,
    B_b1: jax.Array,
    B_w2: jax.Array,
):
    del B_x
    hbm = pl.BlockSpec(memory_space=pl.ANY)
    out_t = pl.pallas_call(
        _kernel,
        in_specs=[hbm] * 6,
        out_specs=hbm,
        out_shape=jax.ShapeDtypeStruct((D, S), bf16),
        scratch_shapes=[
            pltpu.VMEM((D, S), bf16),
            pltpu.VMEM((D, 3 * D), bf16),
            pltpu.VMEM((D, D), bf16),
            pltpu.VMEM((D, F), bf16),
            pltpu.VMEM((F // 128, 128), bf16),
            pltpu.VMEM((D, F), bf16),
            pltpu.VMEM((S // 2, D), i32),
            pltpu.VMEM((D, S), f32),
            pltpu.VMEM((S // 2, F1), i32),
            pltpu.VMEM((3, 5, 640, 128), f32),
            pltpu.VMEM((5, 3 * D, 128), bf16),
            pltpu.VMEM((5, D, 128), f32),
            pltpu.VMEM((D // 2, 640), i32),
            pltpu.VMEM((14, HALO + T, 128), f32),
            pltpu.VMEM((T, 640), f32),
            pltpu.VMEM((D, S), bf16),
            pltpu.VMEM((5, NG, 256, 128), bf16),
            pltpu.VMEM((5, NG, HD, 128), bf16),
            pltpu.VMEM((5, 2, 768, 128), bf16),
            pltpu.VMEM((2 * NG, 80, 128), bf16),
            pltpu.VMEM((len(L2_PRE), 5, NG // 2, 144, 128), bf16),
            pltpu.VMEM((7, NG, HT, 128), bf16),
            pltpu.VMEM((7, 5, NG // 2, 128, 128), bf16),
            pltpu.SMEM((1,), i32),
            pltpu.SemaphoreType.DMA((8 + NTILE,)),
            pltpu.SemaphoreType.DMA((NTILE * NOD,)),
        ],
        compiler_params=pltpu.CompilerParams(vmem_limit_bytes=100 * 1024 * 1024),
    )(A_x.reshape(S, D).T, A_wqkv, A_wo, B_w1, B_b1.reshape(F // 128, 128), B_w2.T)
    return out_t.T.reshape(1, S, D)
```
